```python
import os as _os
_os.environ.setdefault("JAX_PLATFORMS", "cpu")
import jax
import jax.numpy as jnp

def _softmax(x, axis=-1):
    return jax.nn.softmax(x, axis=axis)
def _gelu(x):
    return jax.nn.gelu(x, approximate=True)
def _silu(x):
    return jax.nn.silu(x)
def _sigmoid(x):
    return jax.nn.sigmoid(x)
def _layernorm(x, axis=-1, eps=1e-5):
    m = jnp.mean(x, axis=axis, keepdims=True)
    v = jnp.var(x, axis=axis, keepdims=True)
    return (x - m) / jnp.sqrt(v + eps)
def _scatter_add(tgt, idx, src, axis=0):
    return tgt.at[idx].add(src)
def _segment_sum(src, seg, n):
    return jax.ops.segment_sum(src, seg, n)
class _Rng:
    def __init__(self, key):
        self._k = key
    def _next(self):
        self._k, sub = jax.random.split(self._k)
        return sub
    def normal(self, shape):
        return jax.random.normal(self._next(), shape, dtype=jnp.bfloat16)
    def randint(self, lo, hi, shape):
        return jax.random.randint(self._next(), shape, lo, hi, dtype=jnp.int32)
    def uniform(self, shape, lo=0.0, hi=1.0):
        return jax.random.uniform(self._next(), shape, jnp.bfloat16, lo, hi)
    def permutation(self, n):
        return jax.random.permutation(self._next(), n)


kernel_name = 'gated_mix__grouped_kv_mqa__glu_gated_reglu__prompt'

def setup_inputs():
    _rng = _Rng(jax.random.key(int.from_bytes(__import__("os").urandom(4), "little")))
    _w = (lambda a: (lambda t: t.astype(jnp.bfloat16) if jnp.issubdtype(t.dtype, jnp.floating) else t)(jnp.asarray(a)))
    def _A_setup():
        B, S, D, H = 1, 2048, 1024, 32
        Dh = D // H
        return {
            "x": _w((lambda *s: _rng.normal(s) * 0.05)(B, S, D)),
            "wq": _w((lambda *s: _rng.normal(s) * 0.2)(D, H * Dh)),
            "wk": _w((lambda *s: _rng.normal(s) * 0.2)(D, Dh)),
            "wv": _w((lambda *s: _rng.normal(s) * 0.05)(D, Dh)),
            "wo": _w((lambda *s: _rng.normal(s) * 0.05)(H * Dh, D)),
        }
    _A_in = _A_setup()

    def _B_setup():
        B, S, D, F = 1, 2048, 1024, 3584
        return {
            "x": _w((lambda *s: _rng.normal(s) * 0.05)(B, S, D)),
            "W_gate": _w((lambda *s: _rng.normal(s) * 0.8)(D, F) * (2.0 / D) ** 0.5),
            "W_up": _w((lambda *s: _rng.normal(s) * 0.8)(D, F) * (2.0 / D) ** 0.5),
            "W_down": _w((lambda *s: _rng.normal(s) * 0.8)(F, D) * (1.0 / F) ** 0.5),
        }
    _B_in = _B_setup()

    return {
        "A_x": _A_in["x"],
        "A_wq": _A_in["wq"],
        "A_wk": _A_in["wk"],
        "A_wv": _A_in["wv"],
        "A_wo": _A_in["wo"],
        "B_x": _B_in["x"],
        "B_W_gate": _B_in["W_gate"],
        "B_W_up": _B_in["W_up"],
        "B_W_down": _B_in["W_down"],
        "gate_w": _w((lambda *s: _rng.normal(s) * 0.05)(1024) * 16.0),
    }

def reference(A_x, A_wq, A_wk, A_wv, A_wo, B_x, B_W_gate, B_W_up, B_W_down, gate_w):
    def _A_ref(x, wq, wk, wv, wo):
        B, S, D = x.shape
        H = 32
        Dh = D // H
        q = (lambda x, *d: x.transpose(*d))((x @ wq).reshape(B, S, H, Dh), 0, 2, 1, 3)
        k = x @ wk
        v = x @ wv
        scores = jnp.einsum("bhqd,bkd->bhqk", q, k) * (Dh ** -0.5)
        p = _softmax(scores, axis=-1)
        o = jnp.einsum("bhqk,bkd->bhqd", p, v)
        return (lambda x, *d: x.transpose(*d))(o, 0, 2, 1, 3).reshape(B, S, H * Dh) @ wo

    def _B_ref(x, W_gate, W_up, W_down):
        gate = jnp.einsum("bsd,df->bsf", x, W_gate)
        up = jnp.einsum("bsd,df->bsf", x, W_up)
        gate = gate * (lambda x, dt: x.astype(dt))(gate > 0, gate.dtype)
        h = gate * up
        return jnp.einsum("bsf,fd->bsd", h, W_down)

    x = A_x
    g = _sigmoid((x * gate_w).sum(-1, keepdims=True))
    a = _A_ref(x, A_wq, A_wk, A_wv, A_wo)
    b = _B_ref(x, B_W_gate, B_W_up, B_W_down)
    return g * a + (1 - g) * b
```

```python
import functools
import jax
import jax.numpy as jnp
from jax import lax
from jax.experimental import pallas as pl
from jax.experimental.pallas import tpu as pltpu

H = 32
LOG2E = 1.4426950408889634
NT = (((1,), (1,)), ((), ()))
F32 = jnp.float32
BF16 = jnp.bfloat16
U32 = jnp.uint32


def mm(a, b):
    return jnp.dot(a, b, preferred_element_type=F32)


def pk(x):
    return pltpu.bitcast(x.astype(BF16), U32)


def upk(x):
    return pltpu.bitcast(x, BF16)


def red8(x, op, r=None, rev=False):
    idx = list(range(x.shape[0] // 8))
    if rev:
        idx = idx[::-1]
    for i in idx:
        v = x[8 * i:8 * i + 8]
        r = v if r is None else op(r, v)
    return r


def lhs_combos(a11, a12, a21, a22):
    return [a11 + a22, a21 + a22, a11, a22, a11 + a12, a21 - a11, a12 - a22]


def rhs_combos(b11, b12, b21, b22):
    return [b11 + b22, b11, b12 - b22, b21 - b11, b22, b11 + b12, b21 + b22]


def rhs_packed(b11, b12, b21, b22):
    c = rhs_combos(*(b.astype(F32) for b in (b11, b12, b21, b22)))
    return [pk(c[0]), pltpu.bitcast(b11, U32), pk(c[2]), pk(c[3]), pltpu.bitcast(b22, U32), pk(c[5]), pk(c[6])]


def lhs_packed(a11, a12, a21, a22):
    c = lhs_combos(*(a.astype(F32) for a in (a11, a12, a21, a22)))
    return [pk(c[0]), pk(c[1]), pltpu.bitcast(a11, U32), pltpu.bitcast(a22, U32), pk(c[4]), pk(c[5]), pk(c[6])]


def strassen(prod, out):
    m7 = prod(6)
    yield m7
    m5 = prod(4)
    c11 = m7 - m5
    yield m5
    m4 = prod(3)
    c11 = c11 + m4
    yield m4
    m2 = prod(1)
    out["c21"] = m4 + m2
    yield m2
    m3 = prod(2)
    out["c12"] = m5 + m3
    c22 = m3 - m2
    yield m3
    m1 = prod(0)
    out["c11"] = c11 + m1
    c22 = c22 + m1
    yield m1
    m6 = prod(5)
    out["c22"] = c22 + m6
    yield m6


def take(gen, n=1):
    r = None
    for _ in range(n):
        r = next(gen, None)
    return r


def drain(gen):
    for _ in gen:
        pass


def make(TQ=256, NJ=4, flags=None, NP1=4, extra=0, slab=32, nb=(3, 3, 2), hs=32, prep_at=0, dord=0):
    S, D, F = 2048, 1024, 3584
    KC = 128
    MB = 128
    Dh = D // H
    hD = D // 2
    NB = S // TQ
    FC = F // NJ
    DC = D // NJ
    HU = 512 // TQ
    NU = H // NJ // HU
    NC = S // KC
    FT = FC // 128
    OT = DC // 128
    NPH = FT // 2
    NP = NPH + OT // 2
    NRB = TQ // (2 * MB)
    PB = 256
    NPB = S // PB

    def kernel(x_hbm, wq_hbm, wkt_hbm, wvt_hbm, wo_hbm, wg_hbm, wu_hbm, wd_hbm, gw_hbm, o_hbm,
               x_s, wq_s, wkt_s, wvt_s, gw_s, wo_s, wg_s, wu_s, wd_s,
               xa_s, wqc_s, wguc_s, wdc_s,
               k_s, vt_s, g_s, qt_s, s_s, ot_s, ha_s, hp_s, acc_s, out_s,
               xsem, qsem, ksem, wsem, osem):
        def x_cp(b):
            return pltpu.make_async_copy(x_hbm.at[pl.ds(b * PB, PB)], x_s.at[pl.ds(b * PB, PB)], xsem.at[b])

        def w_cps(j):
            return [
                pltpu.make_async_copy(wg_hbm.at[:, pl.ds(j * FC, FC)], wg_s.at[j], wsem.at[4 * j]),
                pltpu.make_async_copy(wu_hbm.at[:, pl.ds(j * FC, FC)], wu_s.at[j], wsem.at[4 * j + 1]),
                pltpu.make_async_copy(wd_hbm.at[pl.ds(j * FC, FC)], wd_s.at[j], wsem.at[4 * j + 2]),
                pltpu.make_async_copy(wo_hbm.at[pl.ds(j * DC, DC)], wo_s.at[j], wsem.at[4 * j + 3]),
            ]

        def o_cp(b):
            return pltpu.make_async_copy(out_s.at[b % 2], o_hbm.at[pl.ds(b * TQ, TQ)], osem.at[b % 2])

        def prep_weights(j, part, nparts, slot):
            r = hD // nparts
            r0 = pl.multiple_of(part * r, r)
            p0 = pl.multiple_of(part * (r // 2), r // 2)
            for i0 in range(0, r, 16):
                for t in range(FT):
                    cs = slice(t * 128, (t + 1) * 128)
                    ld = lambda ref, o: ref[j, pl.ds(r0 + o + i0, 16), cs]
                    for i, c in enumerate(rhs_packed(ld(wg_s, 0), ld(wu_s, 0), ld(wg_s, hD), ld(wu_s, hD))):
                        wguc_s[slot, i, pl.ds(p0 + i0 // 2, 8), cs] = c
                    yield c
            r = 128 // nparts
            r0 = pl.multiple_of(part * r, r)
            p0 = pl.multiple_of(part * (r // 2), r // 2)
            for p in range(NP):
                ref, t = (wd_s, 2 * p) if p < NPH else (wo_s, 2 * (p - NPH))
                for i0 in range(0, r, 16):
                    for n in range(hD // 128):
                        ld = lambda tt, o: ref[j, pl.ds(tt * 128 + r0 + i0, 16), o + n * 128:o + (n + 1) * 128]
                        for i, c in enumerate(rhs_packed(ld(t, 0), ld(t, hD), ld(t + 1, 0), ld(t + 1, hD))):
                            wdc_s[slot, i, pl.ds(p * 64 + p0 + i0 // 2, 8), n * 128:(n + 1) * 128] = c
                        yield c

        q_cp = pltpu.make_async_copy(wq_hbm, wq_s, qsem)
        small = [pltpu.make_async_copy(wkt_hbm, wkt_s, ksem.at[0]),
                 pltpu.make_async_copy(wvt_hbm, wvt_s, ksem.at[1]),
                 pltpu.make_async_copy(gw_hbm, gw_s, ksem.at[2])]
        q_cp.start()
        x_cp(0).start()
        for c in small:
            c.start()
        q_cp.wait()
        for b in range(1, NPB):
            x_cp(b).start()
        for c in w_cps(0):
            c.start()
        for n in range(hD // 128):
            for i0 in range(0, hD, 16):
                ld = lambda ro, co: wq_s[ro + i0:ro + i0 + 16, co + n * 128:co + (n + 1) * 128]
                for i, c in enumerate(rhs_packed(ld(0, 0), ld(0, hD), ld(hD, 0), ld(hD, hD))):
                    wqc_s[i, i0 // 2:i0 // 2 + 8, n * 128:(n + 1) * 128] = c
        for c in small:
            c.wait()

        def pro(b, carry, prep=False):
            x_cp(b).wait()
            r0 = pl.multiple_of(b * PB, PB)
            side = prep_weights(0, b - NP1, NPB - NP1, 0) if prep else iter(())
            nside = -(-(hD // 16 * FT + NP * 8 * 4) // (NPB - NP1) // 28)
            xb = x_s[pl.ds(r0, PB), :]
            w = jnp.concatenate([wkt_s[...], wvt_s[...], jnp.broadcast_to(gw_s[...], (16, D))], axis=0)
            kvz = lax.dot_general(w, xb, NT, preferred_element_type=F32)
            for n in range(hD // 128):
                for i0 in range(0, MB, 16):
                    ld = lambda ro, co: x_s[pl.ds(r0 + ro + i0, 16), co + n * 128:co + (n + 1) * 128]
                    for i, c in enumerate(lhs_packed(ld(0, 0), ld(0, hD), ld(MB, 0), ld(MB, hD))):
                        xa_s[b, i, i0 // 2:i0 // 2 + 8, n * 128:(n + 1) * 128] = c
            for i in range(PB // 128):
                vt_s[2 * b + i] = pk(kvz[Dh:2 * Dh, i * 128:(i + 1) * 128])
            kt = jnp.concatenate([kvz[0:Dh] * (Dh ** -0.5 * LOG2E), jnp.zeros((128 - Dh, PB), F32)], axis=0)
            k_s[pl.ds(pl.multiple_of(b * (PB // 2), PB // 2), PB // 2), :] = pk(kt.T)
            g = jax.nn.sigmoid(kvz[2 * Dh:2 * Dh + 1])
            g_s[pl.ds(r0, PB), :] = jnp.broadcast_to(g, (128, PB)).T
            for n in range(hD // 128):
                cs = slice(n * 128, (n + 1) * 128)
                out = {}
                dst = {"c11": (0, n), "c12": (0, n + 4), "c21": (1, n), "c22": (1, n + 4)}
                for _ in strassen(lambda r: mm(upk(xa_s[b, r]), upk(wqc_s[r, :, cs])), out):
                    for key in list(out):
                        hh, nn = dst[key]
                        qt_s[2 * b + hh, nn * 64:(nn + 1) * 64, :] = pk(out.pop(key).T)
                    v = take(side, nside)
                    if v is not None:
                        wqc_s[7, pl.ds(pl.multiple_of((b >> 10) * 8, 8), 8), 0:128] = v
            drain(side)
            return carry

        lax.fori_loop(0, NP1, pro, 0)
        for c in w_cps(0):
            c.wait()
        for j in range(1, NJ):
            for c in w_cps(j):
                c.start()
        lax.fori_loop(NP1, NPB, functools.partial(pro, prep=True), 0)
        for c in w_cps(1):
            c.wait()

        def step(it, carry):
            j = it // NB
            b = it % NB

            for jj in range(2, NJ):
                @pl.when(it == (jj - 1) * NB)
                def _():
                    for c in w_cps(jj):
                        c.wait()

            @pl.when(jnp.logical_and(j == NJ - 1, b >= 2))
            def _():
                o_cp(b - 2).wait()

            r0 = pl.multiple_of(b * TQ, TQ)
            st_off = pl.multiple_of((it >> 12) * 8, 8)
            ld_off = pl.multiple_of((j >> 10) * 8, 8)
            wslot = j & 1
            ns = KC // slab

            def qk_mm(u, c):
                h0 = pl.multiple_of((j * NU + u) * HU * (Dh // 2), HU * (Dh // 2))
                rhs = jnp.concatenate(
                    [upk(qt_s[b * (TQ // 128) + t, pl.ds(h0 + i * (Dh // 2), Dh // 2), :])
                     for i in range(HU) for t in range(TQ // 128)], axis=1)
                kk = upk(k_s[c * KC // 2:(c + 1) * KC // 2, :])[:, 0:Dh]
                return mm(kk, rhs)

            def s_load(u, c, i):
                return s_s[pl.ds(ld_off + (u % 2) * S + c * KC + i * slab, slab), :]

            def s_store(u, c, i, s):
                s_s[pl.ds(st_off + (u % 2) * S + c * KC + i * slab, slab), :] = s[i * slab:(i + 1) * slab]

            def fence(v):
                s_s[pl.ds(st_off + 2 * S, 8), 0:128] = v

            def exp_slab(s, mb, l):
                p = jnp.exp2(s - jnp.concatenate([mb] * (slab // 8), axis=0))
                return p, red8(p, jnp.add, l, rev=True)

            def fin_max(m):
                return jnp.broadcast_to(jnp.max(m, axis=0, keepdims=True), m.shape)

            def fin_o(u, l, o):
                ls = jnp.sum(l, axis=0, keepdims=True)
                on = o * (1.0 / ls)
                for i in range(HU):
                    ot_s[(u * HU + i) * Dh:(u * HU + i + 1) * Dh, :] = on[:, i * TQ:(i + 1) * TQ]

            def gu_stream():
                keep = {}
                for t in list(range(2 * NPH, FT)) + list(range(2 * NPH)):
                    for rb in range(NRB):
                        cs = slice(t * 128, (t + 1) * 128)
                        w0 = r0 + rb * 2 * MB
                        out = {}
                        g = strassen(lambda r: mm(upk(xa_s[b * NRB + rb, r]), upk(wguc_s[wslot, r, :, cs])), out)
                        for i in range(6):
                            yield next(g)
                        last = next(g)
                        for i0 in range(0, MB, hs):
                            rs = slice(i0, i0 + hs)
                            ht = jnp.maximum(out["c11"][rs], 0.0) * out["c12"][rs] * (1.0 - g_s[pl.ds(w0 + i0, hs), :])
                            hb = jnp.maximum(out["c21"][rs], 0.0) * out["c22"][rs] * (1.0 - g_s[pl.ds(w0 + MB + i0, hs), :])
                            ps = slice(i0 // 2, (i0 + hs) // 2)
                            if t >= 2 * NPH:
                                hp_s[rb, 0, ps, :] = pk(ht)
                                hp_s[rb, 1, ps, :] = pk(hb)
                            elif t % 2 == 0:
                                keep[rb, i0] = (ht, hb)
                            else:
                                h1t, h1b = keep.pop((rb, i0))
                                for i, c in enumerate(lhs_combos(h1t, ht, h1b, hb)):
                                    ha_s[rb, i, ps, (t // 2) * 128:(t // 2 + 1) * 128] = pk(c)
                        yield last

            def o_lhs():
                for rb in range(NRB):
                    w0 = r0 + rb * 2 * MB
                    blk = lambda t, hh: ot_s[t * 128:(t + 1) * 128, (2 * rb + hh) * MB:(2 * rb + hh + 1) * MB].T
                    for p in range(OT // 2):
                        q4 = [blk(2 * p, 0), blk(2 * p + 1, 0), blk(2 * p, 1), blk(2 * p + 1, 1)]
                        for i0 in range(0, MB, hs):
                            rs = slice(i0, i0 + hs)
                            gt = g_s[pl.ds(w0 + i0, hs), :]
                            gb = g_s[pl.ds(w0 + MB + i0, hs), :]
                            cb = lhs_combos(q4[0][rs] * gt, q4[1][rs] * gt, q4[2][rs] * gb, q4[3][rs] * gb)
                            for i, c in enumerate(cb):
                                ha_s[rb, i, i0 // 2:(i0 + hs) // 2, (NPH + p) * 128:(NPH + p + 1) * 128] = pk(c)

            def down_plain(n, rb, hh):
                cs = slice(n * 512, (n + 1) * 512)
                w0 = r0 + (2 * rb + hh) * MB
                d = mm(upk(hp_s[rb, hh]), wd_s[j, 2 * NPH * 128:, cs])
                prev = acc_s[pl.ds(w0, MB), cs]
                acc_s[pl.ds(w0, MB), cs] = jnp.where(j == 0, 0.0, prev) + d

            def down(n, rb):
                cs = slice(n * 128, (n + 1) * 128)
                out = {}
                dst = {"c11": (0, n), "c12": (0, n + 4), "c21": (1, n), "c22": (1, n + 4)}
                for _ in strassen(lambda r: mm(upk(ha_s[rb, r]), upk(wdc_s[wslot, r, :, cs])), out):
                    for key in list(out):
                        hh, nn = dst[key]
                        w0 = (2 * rb + hh) * MB
                        cc = slice(nn * 128, (nn + 1) * 128)
                        prev = acc_s[pl.ds(r0 + w0, MB), cc]
                        if FT % 2 == 0:
                            prev = jnp.where(j == 0, 0.0, prev)
                        r = prev + out.pop(key)
                        acc_s[pl.ds(r0 + w0, MB), cc] = r
                        out_s[b % 2, w0:w0 + MB, cc] = r.astype(BF16)

            gu = gu_stream()
            ngu = 7 * FT * NRB
            side = prep_weights((j + 1) % NJ, b, NB, 1 - wslot)
            nside = -(-(hD // 16 * FT + NP * 8 * 4) // NB // (NC - 2))
            spare = ngu - NC - nb[0] - (NU - 1) * nb[1] - nb[2]
            nslots = (NU - 1) * (NC - 1)
            mb = None
            slot_i = 0
            for ph in range(NU + 1):
                m = None; l = None; o = None
                if ph > 0:
                    parts = []
                    for i in range(ns):
                        p, l = exp_slab(s_load(ph - 1, 0, ns - 1 - i), mb, l)
                        parts.append(p)
                for c in range(NC):
                    if ph > 0:
                        pcur = jnp.concatenate(parts[::-1], axis=0).astype(BF16)
                        parts = []
                    if ph < NU:
                        s = qk_mm(ph, c)
                    else:
                        s = take(gu)
                    for i in range(ns):
                        if ph > 0 and c + 1 < NC:
                            p, l = exp_slab(s_load(ph - 1, c + 1, ns - 1 - i), mb, l)
                            parts.append(p)
                        if ph < NU:
                            s_store(ph, c, i, s)
                            m = red8(s[i * slab:(i + 1) * slab], jnp.maximum, m)
                        elif c + 1 < NC:
                            fence(s[(i + 1) * slab - 8:(i + 1) * slab])
                    if ph > 0:
                        d = mm(upk(vt_s[c]), pcur)
                        o = d if o is None else o + d
                    if ph == 0:
                        v = take(side, nside)
                        if v is not None:
                            k_s[pl.ds(st_off + S // 2, 8), :] = v
                    if 0 < ph < NU and c + 1 < NC:
                        slot_i += 1
                        take(gu, (slot_i * spare) // nslots - ((slot_i - 1) * spare) // nslots)
                if ph == 0:
                    drain(side)
                if ph > 0:
                    fin_o(ph - 1, l, o)
                if ph < NU:
                    mb = fin_max(m)
                    take(gu, nb[0] if ph == 0 else nb[1])
            o_lhs()
            drain(gu)
            if FT % 2:
                for n in range(2):
                    for rb in range(NRB):
                        for hh in range(2):
                            down_plain(n, rb, hh)
            for n in range(4):
                for rb in range(NRB):
                    down(n, rb)

            @pl.when(j == NJ - 1)
            def _():
                o_cp(b).start()

            return carry

        if extra:
            lax.fori_loop(0, NB * NJ + extra, lambda it, c: step(jnp.where(it < 1 + extra, 1, it - extra), c), 0)
        else:
            lax.fori_loop(0, NB * NJ, step, 0)
        o_cp(NB - 2).wait()
        o_cp(NB - 1).wait()

    def fn(A_x, A_wq, A_wk, A_wv, A_wo, B_x, B_W_gate, B_W_up, B_W_down, gate_w):
        x = A_x.reshape(S, D)
        anyspec = pl.BlockSpec(memory_space=pl.ANY)
        out = pl.pallas_call(
            kernel,
            in_specs=[anyspec] * 9,
            out_specs=anyspec,
            out_shape=jax.ShapeDtypeStruct((S, D), A_x.dtype),
            scratch_shapes=[
                pltpu.VMEM((S, D), BF16),
                pltpu.VMEM((D, D), BF16),
                pltpu.VMEM((Dh, D), BF16),
                pltpu.VMEM((Dh, D), BF16),
                pltpu.VMEM((1, D), BF16),
                pltpu.VMEM((NJ, DC, D), BF16),
                pltpu.VMEM((NJ, D, FC), BF16),
                pltpu.VMEM((NJ, D, FC), BF16),
                pltpu.VMEM((NJ, FC, D), BF16),
                pltpu.VMEM((S // (2 * MB), 7, MB // 2, D // 2), U32),
                pltpu.VMEM((8, D // 4, D // 2), U32),
                pltpu.VMEM((2, 7, D // 4, FC), U32),
                pltpu.VMEM((2, 7, NP * 64, D // 2), U32),
                pltpu.VMEM((S // 2 + 16, 128), U32),
                pltpu.VMEM((S // 128, Dh // 2, 128), U32),
                pltpu.VMEM((S, 128), F32),
                pltpu.VMEM((S // 128, D // 2, 128), U32),
                pltpu.VMEM((2 * S + 16, 512), F32),
                pltpu.VMEM((DC, TQ), F32),
                pltpu.VMEM((NRB, 7, MB // 2, NP * 128), U32),
                pltpu.VMEM((NRB, 2, MB // 2, 128), U32),
                pltpu.VMEM((S, D), F32),
                pltpu.VMEM((2, TQ, D), BF16),
                pltpu.SemaphoreType.DMA((NPB,)),
                pltpu.SemaphoreType.DMA(()),
                pltpu.SemaphoreType.DMA((3,)),
                pltpu.SemaphoreType.DMA((4 * NJ,)),
                pltpu.SemaphoreType.DMA((2,)),
            ],
            compiler_params=pltpu.CompilerParams(vmem_limit_bytes=120 * 2**20, flags=flags),
            name="mainkern",
        )(x, A_wq, A_wk.T, A_wv.T, A_wo, B_W_gate, B_W_up, B_W_down, gate_w.reshape(1, D))
        return out.reshape(A_x.shape)
    return fn


@jax.jit
def pallas_gated_mix__grouped_kv_mqa__glu_gated_reglu__prompt_kernel(
    A_x, A_wq, A_wk, A_wv, A_wo, B_x, B_W_gate, B_W_up, B_W_down, gate_w
):
    return make()(A_x, A_wq, A_wk, A_wv, A_wo, B_x, B_W_gate, B_W_up, B_W_down, gate_w)
```

```python
import contextlib
import functools
import jax
import jax.numpy as jnp
from jax import lax
from jax.experimental import pallas as pl
from jax.experimental.pallas import tpu as pltpu

H = 32
LOG2E = 1.4426950408889634
NT = (((1,), (1,)), ((), ()))
F32 = jnp.float32
BF16 = jnp.bfloat16
U32 = jnp.uint32


def mm(a, b):
    return jnp.dot(a, b, preferred_element_type=F32)


def pk(x):
    return pltpu.bitcast(x.astype(BF16), U32)


def upk(x):
    return pltpu.bitcast(x, BF16)


def red8(x, op, r=None, rev=False):
    idx = list(range(x.shape[0] // 8))
    if rev:
        idx = idx[::-1]
    for i in idx:
        v = x[8 * i:8 * i + 8]
        r = v if r is None else op(r, v)
    return r


ADD, SUB = jnp.add, jnp.subtract
LEFT = ((ADD, 0, 3), (ADD, 2, 3), (None, 0, 0), (None, 3, 3), (ADD, 0, 1), (SUB, 2, 0), (SUB, 1, 3))
RIGHT = ((ADD, 0, 3), (None, 0, 0), (SUB, 1, 3), (SUB, 2, 0), (None, 3, 3), (ADD, 0, 1), (ADD, 2, 3))
USES = (((0, 1), (3, 1)), ((2, 1), (3, -1)), ((1, 1), (3, 1)), ((0, 1), (2, 1)), ((0, -1), (1, 1)), ((3, 1),), ((0, 1),))
ORDER = (6, 4, 3, 2, 1, 0, 5)
SWAP = (2, 4, 5, 6)


def operand(table, i, n, load):
    op, x, y = table[i]
    h = n // 2
    at = lambda q, r, c: load(q // 2 * h + r, q % 2 * h + c)
    if op is None:
        return [[at(x, r, c) for c in range(h)] for r in range(h)]
    return [[op(at(x, r, c).astype(F32), at(y, r, c).astype(F32)) for c in range(h)] for r in range(h)]


def operands(table, n, load, before=None):
    for i in range(7):
        if before and n == 4:
            before()
        g = operand(table, i, n, load)
        if n == 2:
            yield i, g[0][0]
        else:
            flip = 1 if table is RIGHT and i in SWAP else 0
            for k, v in operands(table, 2, lambda r, c: g[r][c ^ flip]):
                yield i * 7 + k, v


def strassen(n, prod, emit, base=0):
    if n == 1:
        m = prod(base)
        emit(0, 0, m)
        yield m
        return
    h = n // 2
    acc = {}
    left = [4, 2, 2, 4]
    for r in ORDER:
        for q, _ in USES[r]:
            left[q] -= 1

        def sink(i, k, m, r=r):
            if n == 4 and r in SWAP:
                k ^= 1
            for q, sign in USES[r]:
                key = (q // 2 * h + i, q % 2 * h + k)
                if key in acc:
                    v = acc.pop(key) + m if sign > 0 else acc.pop(key) - m
                else:
                    assert sign > 0
                    v = m
                if left[q] == 0:
                    emit(key[0], key[1], v)
                else:
                    acc[key] = v

        yield from strassen(h, prod, sink, base * 7 + r)


def make(FTS=(0, 10, 10, 8), OTS=(0, 2, 2, 4), HS=(8, 8, 8, 8), flags=None, NQ=4, slab=32, hs=16,
         wa=1.0, wg=0.0, wd=1.0, mg=300, lag=2, only=None, reps=1, force=False,
         dma=2, mq=14, pr=64, pr2=40, scopes=False, ahead=1, UN=(2, 1, 1, 1), head=1, endlag=4, mix=3, unp=6):
    scope = jax.named_scope if scopes else (lambda n: contextlib.nullcontext())
    S, D, F = 2048, 1024, 3584
    KC = 128
    TQ = 256
    G = 4
    NPR = 49
    Dh = D // H
    NB = S // TQ
    NJ = len(FTS)
    assert sum(FTS) * 128 == F and sum(OTS) * 128 == D and sum(HS) == H
    F0 = [sum(FTS[:j]) * 128 for j in range(NJ)]
    O0 = [sum(OTS[:j]) for j in range(NJ)]
    H0 = [sum(HS[:j]) for j in range(NJ + 1)]
    FM = max(FTS)
    HU = 512 // TQ
    NC = S // KC
    MB = TQ // G
    KG = D // G
    KDS = [(FTS[j] + OTS[j]) // G for j in range(NJ)]
    KM = max(KDS)
    RD = KM * G * 128

    def kernel(x_hbm, wq_hbm, wkt_hbm, wvt_hbm, wo_hbm, wg_hbm, wu_hbm, wd_hbm, gw_hbm, o_hbm,
               x_s, wq_s, wkt_s, wvt_s, gw_s, qh_s,
               wg_s, wu_s, wd_s, xa_s, wguc_a, wguc_b, wdc_a, wdc_b,
               k_s, vt_s, g_s, qt_s, of_s, s_s, nrm_s, ha_s, hb_s, hf_s, acc_s, out_s, z_s,
               xsem, qsem, ksem, wsem, osem):
        wguc = (wguc_a, wguc_b)
        wdc = (wdc_a, wdc_b)
        wqc_s = wguc_a

        def w_cps(j):
            fc = FTS[j] * 128
            return [
                pltpu.make_async_copy(wg_hbm.at[:, pl.ds(F0[j], fc)], wg_s.at[pl.ds(j % 2 * D, D), pl.ds(0, fc)],
                                      wsem.at[4 * j]),
                pltpu.make_async_copy(wu_hbm.at[:, pl.ds(F0[j], fc)], wu_s.at[pl.ds(j % 2 * D, D), pl.ds(0, fc)],
                                      wsem.at[4 * j + 1]),
                pltpu.make_async_copy(wd_hbm.at[pl.ds(F0[j], fc)], wd_s.at[pl.ds(j % 2 * RD, fc)],
                                      wsem.at[4 * j + 2]),
                pltpu.make_async_copy(wo_hbm.at[pl.ds(O0[j] * 128, OTS[j] * 128)],
                                      wd_s.at[pl.ds(j % 2 * RD + fc, OTS[j] * 128)], wsem.at[4 * j + 3])]

        def x_cp(b):
            return pltpu.make_async_copy(x_hbm.at[pl.ds(b * TQ, TQ)], x_s.at[pl.ds(b * TQ, TQ)], xsem.at[b])

        QR = KG // NQ

        def q_cps(p):
            return [pltpu.make_async_copy(wq_hbm.at[pl.ds(k * KG + p * QR, QR)],
                                          wq_s.at[pl.ds(k * KG + p * QR, QR)], qsem.at[p * G + k])
                    for k in range(G)]

        def o_cp(b):
            return pltpu.make_async_copy(out_s.at[b % 2], o_hbm.at[pl.ds(b * TQ, TQ)], osem.at[b % 2])

        def make_pin(latest):
            def pin(ref):
                ref[pl.ds(pl.multiple_of(z_s[0], 8) + ref.shape[0] - 32, 8), 0:128] = latest[0].astype(ref.dtype)
            return pin

        def prep_block(table, load, store, before):
            for i, v in operands(table, G, load, before):
                get = store(i, pk(v))
                if i % 7 == 6:
                    yield get

        def storer(dst, row, t):
            def store(i, v):
                dst[i, pl.ds(row, 8), t * 128:(t + 1) * 128] = v
                return lambda z: dst[i + z, pl.ds(row, 8), t * 128:(t + 1) * 128]
            return store

        def prep_wq(p, carry):
            for c in q_cps(p):
                c.wait()

            @pl.when(p + ahead + 1 < NQ)
            def _():
                for c in q_cps(p + ahead + 1):
                    c.start()

            @pl.when(p + ahead + 1 == NQ)
            def _():
                x_cp(1).start()
                for c in small:
                    c.start()

            r0 = pl.multiple_of(p * QR, QR)
            p0 = pl.multiple_of(p * (QR // 2), QR // 2)
            for i0 in range(0, QR, 16):
                for n in range(KG // 128):
                    load = lambda k, c: wq_s[pl.ds(r0 + k * KG + i0, 16), c * KG + n * 128:c * KG + (n + 1) * 128]
                    for _ in prep_block(RIGHT, load, storer(wqc_s, p0 + i0 // 2, n), None):
                        pass
            return carry

        def prep_x(b, before):
            r0 = pl.multiple_of(b * TQ, TQ)
            for n in range(KG // 128):
                for i0 in range(0, MB, 16):
                    load = lambda r, c: x_s[pl.ds(r0 + r * MB + i0, 16), c * KG + n * 128:c * KG + (n + 1) * 128]

                    def store(i, v):
                        xa_s[b, i, i0 // 2:i0 // 2 + 8, n * 128:(n + 1) * 128] = v
                        return lambda z: xa_s[b, i + z, i0 // 2:i0 // 2 + 8, n * 128:(n + 1) * 128]
                    yield from prep_block(LEFT, load, store, before)

        def keys_values(b):
            r0 = pl.multiple_of(b * TQ, TQ)
            gw = gw_s[0:8, :].astype(F32)
            gw = jnp.concatenate([jnp.broadcast_to(gw[i:i + 1], (16, 128)) for i in range(D // 128)], axis=1)
            w = jnp.concatenate([wkt_s[...], wvt_s[...], gw.astype(BF16)], axis=0)
            kvz = lax.dot_general(w, x_s[pl.ds(r0, TQ), :], NT, preferred_element_type=F32)
            for i in range(TQ // 128):
                vt_s[2 * b + i] = pk(kvz[Dh:2 * Dh, i * 128:(i + 1) * 128])
            kt = kvz[0:Dh] * (Dh ** -0.5 * LOG2E)
            nrm_s[1] = jnp.maximum(nrm_s[1], jnp.sum(kt * kt, axis=0, keepdims=True))
            nrm_s[2] = red8(jnp.abs(kvz[Dh:2 * Dh]), jnp.maximum, nrm_s[2])
            kt = jnp.concatenate([kt, jnp.zeros((128 - Dh, TQ), F32)], axis=0)
            k_s[pl.ds(pl.multiple_of(b * (TQ // 2), TQ // 2), TQ // 2), :] = pltpu.bitcast(kt.astype(BF16).T, U32)
            g = jax.nn.sigmoid(kvz[2 * Dh:2 * Dh + 1])
            g_s[pl.ds(r0, TQ), :] = jnp.broadcast_to(g, (128, TQ)).T

        def queries(b, prep):
            latest = [None]
            pin = make_pin(latest)
            side = prep_x(b + 1, lambda: pin(x_s)) if prep else iter(())
            nside = KG // 128 * (MB // 16) * 7 if prep else 0
            done = [0, 0]
            st = [nrm_s[0, :, 0:128]]

            def put_q(row, hh, nn, q):
                qt = q.astype(BF16).T
                qt_s[row, nn * 64:(nn + 1) * 64, :] = pltpu.bitcast(qt, U32)
                qf = qt.astype(F32)
                of_s[row // 2, nn * 128:(nn + 1) * 128, hh * 128:(hh + 1) * 128] = qf
                q2 = qf * qf
                for i in range(128 // Dh):
                    st[0] = jnp.maximum(
                        st[0], jnp.sum(red8(q2[i * Dh:(i + 1) * Dh], jnp.add), axis=0, keepdims=True))
                nrm_s[0, :, 0:128] = st[0]

            keys_values(b)
            for i in range(2):
                put_q(jnp.where(b == 0, S // 128, 2 * b - 1), 1, 5 + 2 * i, qh_s[i])
            for n in range(KG // 128):
                blocks = {}
                per = 128 // MB

                def emit(r, c, v):
                    blocks[r, c] = v
                    h0 = r // per * per
                    if all((h0 + i, c) in blocks for i in range(per)):
                        q = jnp.concatenate([blocks.pop((h0 + i, c)) for i in range(per)], axis=0)
                        if prep and n == 1 and r >= 2 and c >= 2:
                            qh_s[c - 2] = q
                        else:
                            put_q(2 * b + r // per, r // per, c * (KG // 128) + n, q)

                for v in strassen(G, lambda i: mm(upk(xa_s[b, i]), upk(wqc_s[i, :, n * 128:(n + 1) * 128])), emit):
                    latest[0] = v[0:8]
                    done[0] += 1
                    while done[1] < min(nside, nside * done[0] // (NPR * (KG // 128) - mq)):
                        qt_s[S // 128 + z_s[0], 0:8, :] = next(side)(z_s[2])
                        done[1] += 1

        small = [pltpu.make_async_copy(wkt_hbm, wkt_s, ksem.at[0]),
                 pltpu.make_async_copy(wvt_hbm, wvt_s, ksem.at[1]),
                 pltpu.make_async_copy(gw_hbm, gw_s.at[pl.ds(0, 8)], ksem.at[2])]
        x_cp(0).start()
        for p in range(ahead):
            for c in q_cps(p):
                c.start()
        for i in range(4):
            z_s[i] = 0
        nrm_s[...] = jnp.zeros(nrm_s.shape, F32)
        qh_s[...] = jnp.zeros(qh_s.shape, F32)
        with scope("s0_wait"):
            x_cp(0).wait()
        for c in q_cps(ahead):
            c.start()
        with scope("s1_kv0"):
            for _ in prep_x(0, None):
                pass
        with scope("s2_wq"):
            lax.fori_loop(0, NQ, prep_wq, 0)
        x_cp(2).start()
        for c in small:
            c.wait()

        def pro(b, carry):
            x_cp(b + 1).wait()

            @pl.when(b == 1)
            def _():
                for k in range(3, NB):
                    x_cp(k).start()

            @pl.when(b == dma)
            def _():
                for c in w_cps(1):
                    c.start()

            queries(b, True)
            return carry

        with scope("s3_pro"):
            lax.fori_loop(0, NB - 1, pro, 0)
        with scope("s4_q7"):
            queries(NB - 1, False)

        def q_rhs(b, h):
            return jnp.concatenate(
                [upk(qt_s[b * (TQ // 128) + t, (h + i) * (Dh // 2):(h + i + 1) * (Dh // 2), :])
                 for i in range(HU) for t in range(TQ // 128)], axis=1)

        bound2 = jnp.max(nrm_s[0]) * jnp.max(nrm_s[1])
        vmax = jnp.max(nrm_s[2])
        safe = (bound2 <= 50.0 ** 2) & (vmax <= 2.0 ** 40) & (vmax >= 2.0 ** -30)
        if force:
            safe = safe & (vmax < 0)

        @pl.when(jnp.logical_not(safe))
        def _():
            def one(i, carry):
                blk, h = i // H, i % H
                q = upk(qt_s[blk, pl.ds(pl.multiple_of(h * (Dh // 2), Dh // 2), Dh // 2), :])
                s = mm(upk(k_s[...])[:, 0:Dh], q)
                p = jnp.exp2(s - jnp.max(s, axis=0, keepdims=True))
                vt = jnp.concatenate([upk(vt_s[c]) for c in range(NC)], axis=1)
                o = mm(vt, p.astype(BF16)) / jnp.sum(p, axis=0, keepdims=True)
                for t in range(TQ // 128):
                    @pl.when(blk % (TQ // 128) == t)
                    def _():
                        of_s[blk // (TQ // 128), pl.ds(pl.multiple_of(h * Dh, Dh), Dh), t * 128:(t + 1) * 128] = o
                return carry

            lax.fori_loop(0, S // 128 * H, one, 0)

        def prep_weights(j, part, pin):
            r = KG // NB
            r0 = pl.multiple_of(part * r, r)
            p0 = pl.multiple_of(part * (r // 2), r // 2)
            for i0 in range(0, r, 16):
                for t in range(FTS[j] // 2):
                    load = lambda k, c: (wg_s, wu_s)[c // 2][
                        pl.ds(j % 2 * D + r0 + k * KG + i0, 16), (t * 2 + c % 2) * 128:(t * 2 + c % 2 + 1) * 128]
                    yield from prep_block(RIGHT, load, storer(wguc[j % 2], p0 + i0 // 2, t),
                                          lambda: (pin(wg_s), pin(wu_s)))
            r = 128 // NB
            r0 = pl.multiple_of(part * r, r)
            p0 = pl.multiple_of(part * (r // 2), r // 2)
            for p in range(KDS[j]):
                for n in range(KG // 128):
                    load = lambda k, c: wd_s[pl.ds(j % 2 * RD + (p * G + k) * 128 + r0, 16),
                                             c * KG + n * 128:c * KG + (n + 1) * 128]
                    yield from prep_block(RIGHT, load, storer(wdc[j % 2], p * 64 + p0, n), lambda: pin(wd_s))

        def step(b, j):
            if only is not None:
                b = b % NB
            last_j = j == NJ - 1
            FT = FTS[j]
            KD = KDS[j]
            first_d = sum(KDS[:j]) == 0
            NU = HS[j] // HU
            KS = KD - 1 if last_j else KD
            r0 = pl.multiple_of(b * TQ, TQ)
            st_off = pl.multiple_of(z_s[0], 8)
            ld_off = pl.multiple_of(z_s[1], 8)
            z2 = z_s[2]

            def fence(v):
                s_s[pl.ds(st_off, 8), 0:128] = v

            c_gu = MB * (KG // 128) // 4
            tot_p = NU * S * wa + NPR * (FT // 2) * c_gu * wg + NPR * (KG // 128) * (MB * KD // 4) * wd
            latest = [None]
            pin = make_pin(latest)
            side = iter(()) if last_j else prep_weights(j + 1, b, pin)
            nside = 0 if last_j else 7 * (KG // NB // 16 * (FTS[j + 1] // 2) + KDS[j + 1] * (KG // 128))
            prog = [0.0, 0, 0.0]
            queue = []
            late = [False]

            def pump(n):
                while n and queue:
                    v = next(queue[0], None)
                    if v is None:
                        queue.pop(0)
                    else:
                        fence(pltpu.bitcast(v, F32))
                        n -= 1

            def tick(v, cyc, w):
                prog[0] += w * cyc
                fence(v)
                latest[0] = v
                while prog[1] < min(nside, int(nside * prog[0] / (tot_p - mg))):
                    fence(pltpu.bitcast(next(side)(z2), F32))
                    prog[1] += 1
                prog[2] += cyc / (pr2 if late[0] else pr)
                pump(int(prog[2]))
                prog[2] -= int(prog[2])

            def left_operands(p):
                dst, q = (ha_s, p) if p < KS else (hb_s, p - KS)
                for i0 in range(0, MB, hs):
                    load = lambda r, k: hf_s[pl.ds(ld_off + r * MB + i0, hs), (p * G + k) * 128:(p * G + k + 1) * 128]
                    for i, v in operands(LEFT, G, load, lambda: pin(hf_s)):
                        dst[i, i0 // 2:(i0 + hs) // 2, q * 128:(q + 1) * 128] = pk(v)
                        if i % 7 == 6:
                            yield dst[i + z2, i0 // 2:i0 // 2 + 8, q * 128:(q + 1) * 128]

            pend = {}

            def put(t, row, v):
                hf_s[pl.ds(st_off + row, v.shape[0]), t * 128:(t + 1) * 128] = v
                p = t // G
                pend[p] = pend.get(p, 0) + v.shape[0]
                if pend[p] == G * TQ:
                    queue.append(left_operands(p))

            def o_tile(t):
                rs = slice((O0[j] + t) * 128, (O0[j] + t + 1) * 128)
                for hh in range(TQ // 128):
                    put(FT + t, hh * 128,
                        of_s[b + z2, rs, hh * 128:(hh + 1) * 128].T * g_s[pl.ds(r0 + hh * 128, 128), :])

            def gate_up(t):
                res = {}

                def emit(r, c, v):
                    res[r, c] = v
                    k = c % 2
                    if (r, k) in res and (r, 2 + k) in res:
                        put(t * 2 + k, r * MB, jnp.maximum(res.pop((r, k)), 0.0) * res.pop((r, 2 + k))
                            * (1.0 - g_s[pl.ds(r0 + r * MB, MB), :]))

                for v in strassen(
                        G, lambda i: mm(upk(xa_s[b, i]), upk(wguc[j % 2][i, :, t * 128:(t + 1) * 128])), emit):
                    tick(v[MB - 8:], c_gu, wg)

            def down(n, ka, kd):
                def emit(r, c, v):
                    cc = slice(c * KG + n * 128, c * KG + (n + 1) * 128)
                    if not first_d or ka > 0:
                        v = acc_s[pl.ds(r0 + r * MB, MB), cc] + v
                    if last_j and kd == KD:
                        out_s[b % 2, r * MB:(r + 1) * MB, cc] = v.astype(BF16)
                    else:
                        acc_s[pl.ds(r0 + r * MB, MB), cc] = v

                lhs = lambda i: jnp.concatenate([ha_s[i + z2, :, 0:KS * 128]] * (ka == 0)
                                                + [hb_s[i + z2, :, 0:(kd - KS) * 128]] * (kd > KS), axis=1)
                for v in strassen(G, lambda i: mm(
                        upk(lhs(i)), upk(wdc[j % 2][i, ka * 64:kd * 64, n * 128:(n + 1) * 128])), emit):
                    tick(v[MB - 8:], MB * (kd - ka) // 4, wd)
                    yield

            steps = [(u, c) for u in range(NU) for c in range(NC)]
            st = {"l": None, "o": None}
            ps = {}

            def scores(u, c):
                kk = jnp.concatenate(
                    [k_s[r // 2:r // 2 + 8, :] for r in range((c + 1) * KC - 16, c * KC - 1, -16)], axis=0)
                s = mm(upk(kk)[:, 0:Dh], q_rhs(b, H0[j] + u * HU))
                for i in range(slab, KC + 1, slab):
                    tick(s[i - 8:i, 0:128], slab, wa)
                p = jnp.exp2(jnp.concatenate([s[i:i + 16] for i in range(KC - 16, -1, -16)], axis=0))
                st["l"] = red8(p, jnp.add, None if c == 0 else st["l"], rev=True)
                ps[u, c] = (p.astype(BF16), st["l"])
                s_s[pl.ds(st_off + 8, 8), :] = st["l"]

            def attend(u, c):
                p, l = ps.pop((u, c))
                d = mm(upk(vt_s[c]), p)
                st["o"] = d if c == 0 else st["o"] + d
                if c == NC - 1:
                    on = st["o"] * (1.0 / jnp.sum(l, axis=0, keepdims=True))
                    for i in range(HU):
                        h = H0[j] + u * HU + i
                        of_s[b, h * Dh:(h + 1) * Dh, :] = jnp.where(
                            safe, on[:, i * TQ:(i + 1) * TQ], of_s[b, h * Dh:(h + 1) * Dh, :])

            early_o = [t for t in range(OTS[j]) if (O0[j] + t + 1) * 128 <= H0[j] * Dh]
            nh = head if FT else 0
            for i in range(nh):
                scores(*steps[i])
            for t in range(FT // 2):
                gate_up(t)
                if t == 0:
                    for k in early_o:
                        o_tile(k)
            dn = [down(0, 0, KS)] if KD else []
            if KS < KD:
                dn += [down(0, KS, KD)]
            dn += [down(n, 0, KD) for n in range(1, KG // 128) if KD]
            done = 0
            for i in range(len(steps)):
                if i >= nh:
                    scores(*steps[i])
                while done + lag <= i < len(steps) - (0 if KD else endlag):
                    attend(*steps[done])
                    done += 1
            for i in range(done, len(steps)):
                if KD:
                    pump(1000)
                    for _ in range(mix):
                        next(dn[0])
                attend(*steps[i])
            late[0] = True
            for t in range(OTS[j]):
                if t not in early_o:
                    o_tile(t)
            for g in dn:
                for _ in g:
                    pass
                pump(1000)
            for _ in side:
                pass

        for j in range(NJ):
            if j + 1 < NJ:
                with scope(f"w{j}"):
                    for c in w_cps(j + 1):
                        c.wait()
            if j + 2 < NJ:
                for c in w_cps(j + 2):
                    c.start()
            if only is None or j == only:
                def body(i, carry):
                    if j == NJ - 1:
                        @pl.when(i >= 2)
                        def _():
                            o_cp((i - 2) % NB).wait()
                    with scope(f"it{j}"):
                        for k in range(UN[j]):
                            step(i * UN[j] + k, j)
                    if j == NJ - 1:
                        o_cp(i % NB).start()
                    return carry

                lax.fori_loop(0, NB * reps // UN[j], body, 0)
        if only is None or only == NJ - 1:
            with scope("z_out"):
                o_cp(NB - 2).wait()
                o_cp(NB - 1).wait()

    def fn(A_x, A_wq, A_wk, A_wv, A_wo, B_x, B_W_gate, B_W_up, B_W_down, gate_w):
        x = A_x.reshape(S, D)
        anyspec = pl.BlockSpec(memory_space=pl.ANY)
        out = pl.pallas_call(
            kernel,
            in_specs=[anyspec] * 9,
            out_specs=anyspec,
            out_shape=jax.ShapeDtypeStruct((S, D), A_x.dtype),
            scratch_shapes=[
                pltpu.VMEM((S + 32, D), BF16),
                pltpu.VMEM((D, D), BF16),
                pltpu.VMEM((Dh, D), BF16),
                pltpu.VMEM((Dh, D), BF16),
                pltpu.VMEM((64, 128), BF16),
                pltpu.VMEM((2, 128, 128), F32),
                pltpu.VMEM((2 * D + 32, FM * 128), BF16),
                pltpu.VMEM((2 * D + 32, FM * 128), BF16),
                pltpu.VMEM((2 * RD + 32, D), BF16),
                pltpu.VMEM((NB, NPR, MB // 2, KG), U32),
                pltpu.VMEM((NPR, KG // 2, FM // 2 * 128), U32),
                pltpu.VMEM((NPR, KG // 2, FM // 2 * 128), U32),
                pltpu.VMEM((NPR, KM * 64, KG), U32),
                pltpu.VMEM((NPR, KM * 64, KG), U32),
                pltpu.VMEM((S // 2, 128), U32),
                pltpu.VMEM((S // 128, Dh // 2, 128), U32),
                pltpu.VMEM((S, 128), F32),
                pltpu.VMEM((S // 128 + 1, D // 2, 128), U32),
                pltpu.VMEM((NB + 1, D, TQ), F32),
                pltpu.VMEM((24, 512), F32),
                pltpu.VMEM((4, 8, TQ), F32),
                pltpu.VMEM((NPR, MB // 2, KM * 128), U32),
                pltpu.VMEM((NPR, MB // 2, 128), U32),
                pltpu.VMEM((TQ + 32, KM * G * 128), F32),
                pltpu.VMEM((S, D), F32),
                pltpu.VMEM((2, TQ, D), BF16),
                pltpu.SMEM((4,), jnp.int32),
                pltpu.SemaphoreType.DMA((NB,)),
                pltpu.SemaphoreType.DMA((NQ * G,)),
                pltpu.SemaphoreType.DMA((3,)),
                pltpu.SemaphoreType.DMA((4 * NJ,)),
                pltpu.SemaphoreType.DMA((2,)),
            ],
            compiler_params=pltpu.CompilerParams(vmem_limit_bytes=127 * 2**20, flags=flags),
            name="mainkern",
        )(x, A_wq, A_wk.T, A_wv.T, A_wo, B_W_gate, B_W_up, B_W_down, gate_w.reshape(D // 128, 128))
        return out.reshape(A_x.shape)
    return fn


@jax.jit
def pallas_gated_mix__grouped_kv_mqa__glu_gated_reglu__prompt_kernel(
    A_x, A_wq, A_wk, A_wv, A_wo, B_x, B_W_gate, B_W_up, B_W_down, gate_w
):
    return make()(A_x, A_wq, A_wk, A_wv, A_wo, B_x, B_W_gate, B_W_up, B_W_down, gate_w)
```

```python
import jax
import jax.numpy as jnp
from jax import lax
from jax.experimental import pallas as pl
from jax.experimental.pallas import tpu as pltpu

F32 = jnp.float32
BF16 = jnp.bfloat16
U32 = jnp.uint32
LOG2E = 1.4426950408889634

S, D, F, H = 2048, 1024, 3584, 32
DH = D // H
TQ = 256
NB = S // TQ
KC = 128
NC = S // KC
HU = 512 // TQ
G = 4
NPROD = 49
MB = TQ // G
KG = D // G

HEADS = (10, 10, 12)
FFN_TILES = (0, 14, 14)
OUT_TILES = (0, 2, 6)
NJ = len(HEADS)
HEAD0 = [sum(HEADS[:j]) for j in range(NJ)]
FFN0 = [sum(FFN_TILES[:j]) for j in range(NJ)]
OUT0 = [sum(OUT_TILES[:j]) for j in range(NJ)]
GROUPS = [(FFN_TILES[j] + OUT_TILES[j]) // G for j in range(NJ)]
FM, GM = max(FFN_TILES), max(GROUPS)
NQ = 4
QR = KG // NQ

ADD, SUB = jnp.add, jnp.subtract
LEFT = ((ADD, 0, 3), (ADD, 2, 3), (None, 0, 0), (None, 3, 3), (ADD, 0, 1), (SUB, 2, 0), (SUB, 1, 3))
RIGHT = ((ADD, 0, 3), (None, 0, 0), (SUB, 1, 3), (SUB, 2, 0), (None, 3, 3), (ADD, 0, 1), (ADD, 2, 3))
USES = (((0, 1), (3, 1)), ((2, 1), (3, -1)), ((1, 1), (3, 1)), ((0, 1), (2, 1)), ((0, -1), (1, 1)),
        ((3, 1),), ((0, 1),))
ORDER = (6, 4, 3, 2, 1, 0, 5)
SWAP = (2, 4, 5, 6)


def mm(a, b):
    return jnp.dot(a, b, preferred_element_type=F32)


def pack(x):
    return pltpu.bitcast(x.astype(BF16), U32)


def unpack(x):
    return pltpu.bitcast(x, BF16)


def tile(i):
    return slice(i * 128, (i + 1) * 128)


def fold8(x, op, r=None, reverse=False):
    groups = range(x.shape[0] // 8)
    for i in reversed(groups) if reverse else groups:
        v = x[8 * i:8 * i + 8]
        r = v if r is None else op(r, v)
    return r


def operands(table, n, load, before=None):
    h = n // 2
    for i, (op, x, y) in enumerate(table):
        if before:
            before()
        at = lambda q, r, c: load(q // 2 * h + r, q % 2 * h + c)
        g = [[op(at(x, r, c).astype(F32), at(y, r, c).astype(F32)) if op else at(x, r, c)
              for c in range(h)] for r in range(h)]
        if h == 1:
            yield i, g[0][0]
        else:
            flip = int(table is RIGHT and i in SWAP)
            for k, v in operands(table, h, lambda r, c: g[r][c ^ flip]):
                yield i * 7 + k, v


def strassen(n, product, emit, base=0):
    if n == 1:
        m = product(base)
        emit(0, 0, m)
        yield m
        return
    h = n // 2
    acc = {}
    left = [4, 2, 2, 4]
    for r in ORDER:
        for q, _ in USES[r]:
            left[q] -= 1

        def sink(i, k, m, r=r):
            if h > 1 and r in SWAP:
                k ^= 1
            for q, sign in USES[r]:
                key = (q // 2 * h + i, q % 2 * h + k)
                if key in acc:
                    v = acc.pop(key) + m if sign > 0 else acc.pop(key) - m
                else:
                    assert sign > 0
                    v = m
                if left[q]:
                    acc[key] = v
                else:
                    emit(key[0], key[1], v)

        yield from strassen(h, product, sink, base * 7 + r)


def drain(gen):
    for _ in gen:
        pass


def kernel(x_hbm, wq_hbm, wkt_hbm, wvt_hbm, wo_hbm, wg_hbm, wu_hbm, wd_hbm, gw_hbm, o_hbm,
           x_s, wq_s, wkt_s, wvt_s, gw_s, qh_s, wg_s, wu_s, wd_s,
           xa_s, wgu_a, wgu_b, wdn_a, wdn_b,
           k_s, vt_s, g_s, qt_s, ot_s, fence_s, norm_s, ha_s, hb_s, hf_s, acc_s, out_s, zero_s,
           x_sem, q_sem, k_sem, w_sem, o_sem):
    wgu = (wgu_a, wgu_b)
    wdn = (wdn_a, wdn_b)
    wqc_s = wgu_a

    def x_copy(b):
        return pltpu.make_async_copy(x_hbm.at[pl.ds(b * TQ, TQ)], x_s.at[pl.ds(b * TQ, TQ)], x_sem.at[b])

    def q_copies(p):
        return [pltpu.make_async_copy(wq_hbm.at[pl.ds(k * KG + p * QR, QR)],
                                      wq_s.at[pl.ds(k * KG + p * QR, QR)], q_sem.at[p * G + k])
                for k in range(G)]

    def w_slot(j, b):
        return jnp.where(b == 0, 2 + j % 2, b % 2)

    def w_copies(j, b):
        fc, slot, r = FFN_TILES[j] * 128, w_slot(j, b), KG // NB
        b = jnp.minimum(b, NB - 1)
        rows = pl.ds(pl.multiple_of(b * r, r), r)
        drows = pl.ds(pl.multiple_of(b * 16, 16), 16)
        return [
            pltpu.make_async_copy(wg_hbm.at[:, rows, pl.ds(FFN0[j] * 128, fc)],
                                  wg_s.at[pl.ds(slot * G, G), :, pl.ds(0, fc)], w_sem.at[4 * slot]),
            pltpu.make_async_copy(wu_hbm.at[:, rows, pl.ds(FFN0[j] * 128, fc)],
                                  wu_s.at[pl.ds(slot * G, G), :, pl.ds(0, fc)], w_sem.at[4 * slot + 1]),
            pltpu.make_async_copy(wd_hbm.at[pl.ds(FFN0[j], FFN_TILES[j]), drows],
                                  wd_s.at[pl.ds(slot * GM * G, FFN_TILES[j])], w_sem.at[4 * slot + 2]),
            pltpu.make_async_copy(wo_hbm.at[pl.ds(OUT0[j], OUT_TILES[j]), drows],
                                  wd_s.at[pl.ds(slot * GM * G + FFN_TILES[j], OUT_TILES[j])],
                                  w_sem.at[4 * slot + 3])]

    def o_copy(b):
        return pltpu.make_async_copy(out_s.at[b % 2], o_hbm.at[pl.ds(b * TQ, TQ)], o_sem.at[b % 2])

    kv_copies = [pltpu.make_async_copy(wkt_hbm, wkt_s, k_sem.at[0]),
                 pltpu.make_async_copy(wvt_hbm, wvt_s, k_sem.at[1]),
                 pltpu.make_async_copy(gw_hbm, gw_s.at[pl.ds(0, 8)], k_sem.at[2])]

    def pin(ref, v):
        if len(ref.shape) == 3:
            ref[zero_s[0] + ref.shape[0] - 1, 0:8, 0:128] = v.astype(ref.dtype)
        else:
            ref[pl.ds(pl.multiple_of(zero_s[0], 8) + ref.shape[0] - 32, 8), 0:128] = v.astype(ref.dtype)

    def operand_pieces(table, load, store, before):
        for i, v in operands(table, G, load, before):
            reread = store(i, pack(v))
            if i % 7 == 6:
                yield reread

    def right_store(dst, row, t):
        def store(i, v):
            dst[i, pl.ds(row, 8), tile(t)] = v
            return lambda z: dst[i + z, pl.ds(row, 8), tile(t)]
        return store

    def prepare_wq(p, carry):
        for c in q_copies(p):
            c.wait()

        @pl.when(p + 2 < NQ)
        def _():
            for c in q_copies(p + 2):
                c.start()

        @pl.when(p + 2 == NQ)
        def _():
            x_copy(1).start()
            for c in kv_copies:
                c.start()

        r0 = pl.multiple_of(p * QR, QR)
        p0 = pl.multiple_of(p * (QR // 2), QR // 2)
        for i0 in range(0, QR, 16):
            for n in range(KG // 128):
                load = lambda k, c: wq_s[pl.ds(r0 + k * KG + i0, 16), tile(c * KG // 128 + n)]
                drain(operand_pieces(RIGHT, load, right_store(wqc_s, p0 + i0 // 2, n), None))
        return carry

    def prepare_x(b, before):
        r0 = pl.multiple_of(b * TQ, TQ)
        for n in range(KG // 128):
            for i0 in range(0, MB, 16):
                load = lambda r, c: x_s[pl.ds(r0 + r * MB + i0, 16), tile(c * KG // 128 + n)]

                def store(i, v):
                    xa_s[b, i, i0 // 2:i0 // 2 + 8, tile(n)] = v
                    return lambda z: xa_s[b, i + z, i0 // 2:i0 // 2 + 8, tile(n)]
                yield from operand_pieces(LEFT, load, store, before)

    def prepare_weights(j, b, pin_latest):
        r = KG // NB
        slot = w_slot(j, b)
        p0 = pl.multiple_of(b * (r // 2), r // 2)
        for i0 in range(0, r, 16):
            for t in range(FFN_TILES[j] // 2):
                load = lambda k, c: (wg_s, wu_s)[c // 2][slot * G + k, i0:i0 + 16, tile(t * 2 + c % 2)]
                yield from operand_pieces(RIGHT, load, right_store(wgu[j % 2], p0 + i0 // 2, t),
                                          lambda: (pin_latest(wg_s), pin_latest(wu_s)))
        p0 = pl.multiple_of(b * 8, 8)
        for p in range(GROUPS[j]):
            for n in range(KG // 128):
                load = lambda k, c: wd_s[slot * GM * G + p * G + k, :, tile(c * KG // 128 + n)]
                yield from operand_pieces(RIGHT, load, right_store(wdn[j % 2], p * 64 + p0, n),
                                          lambda: pin_latest(wd_s))

    def keys_values(b):
        r0 = pl.multiple_of(b * TQ, TQ)
        gw = gw_s[0:8, :].astype(F32)
        gw = jnp.concatenate([jnp.broadcast_to(gw[i:i + 1], (16, 128)) for i in range(D // 128)], axis=1)
        w = jnp.concatenate([wkt_s[...], wvt_s[...], gw.astype(BF16)], axis=0)
        kvz = lax.dot_general(w, x_s[pl.ds(r0, TQ), :], (((1,), (1,)), ((), ())),
                              preferred_element_type=F32)
        for i in range(TQ // 128):
            vt_s[2 * b + i] = pack(kvz[DH:2 * DH, tile(i)])
        kt = kvz[0:DH] * (DH ** -0.5 * LOG2E)
        norm_s[1] = jnp.maximum(norm_s[1], jnp.sum(kt * kt, axis=0, keepdims=True))
        norm_s[2] = fold8(jnp.abs(kvz[DH:2 * DH]), jnp.maximum, norm_s[2])
        kt = jnp.concatenate([kt, jnp.zeros((128 - DH, TQ), F32)], axis=0)
        k_s[pl.ds(pl.multiple_of(b * (TQ // 2), TQ // 2), TQ // 2), :] = pltpu.bitcast(kt.astype(BF16).T, U32)
        g = jax.nn.sigmoid(kvz[2 * DH:2 * DH + 1])
        g_s[pl.ds(r0, TQ), :] = jnp.broadcast_to(g, (128, TQ)).T

    def projections(b, last):
        latest = [None]
        side = iter(()) if last else prepare_x(b + 1, lambda: pin(x_s, latest[0]))
        n_side = 0 if last else KG // 128 * (MB // 16) * 7
        norm = [norm_s[0, :, 0:128]]

        def put_q(row, half, t, q):
            qt = q.astype(BF16).T
            qt_s[row, t * 64:(t + 1) * 64, :] = pltpu.bitcast(qt, U32)
            qf = qt.astype(F32)
            ot_s[row // 2, tile(t), tile(half)] = qf
            q2 = qf * qf
            for i in range(128 // DH):
                n2 = jnp.sum(fold8(q2[i * DH:(i + 1) * DH], jnp.add), axis=0, keepdims=True)
                norm[0] = jnp.maximum(norm[0], n2)
            norm_s[0, :, 0:128] = norm[0]

        if last:
            keys_values(b)
        for i in range(2):
            put_q(jnp.maximum(2 * b - 1, 1), 1, 5 + 2 * i, qh_s[i])
        products = pieces = 0
        for n in range(KG // 128):
            blocks = {}

            def emit(r, c, v):
                blocks[r, c] = v
                top = r // 2 * 2
                if (top, c) in blocks and (top + 1, c) in blocks:
                    q = jnp.concatenate([blocks.pop((top, c)), blocks.pop((top + 1, c))], axis=0)
                    if not last and n == 1 and r >= 2 and c >= 2:
                        qh_s[c - 2] = q
                    else:
                        put_q(2 * b + r // 2, r // 2, c * KG // 128 + n, q)

            for v in strassen(G, lambda i: mm(unpack(xa_s[b, i]), unpack(wqc_s[i, :, tile(n)])), emit):
                latest[0] = v[0:8]
                products += 1
                if not last and products == 4:
                    keys_values(b)
                while pieces < min(n_side, n_side * (products - 4) // (NPROD * (KG // 128) - 12)):
                    qt_s[S // 128 + zero_s[0], 0:8, :] = next(side)(zero_s[2])
                    pieces += 1

    x_copy(0).start()
    for c in q_copies(0):
        c.start()
    for i in range(4):
        zero_s[i] = 0
    norm_s[...] = jnp.zeros(norm_s.shape, F32)
    qh_s[...] = jnp.zeros(qh_s.shape, F32)
    x_copy(0).wait()
    for c in q_copies(1):
        c.start()
    drain(prepare_x(0, None))
    lax.fori_loop(0, NQ, prepare_wq, 0)
    x_copy(2).start()
    for c in kv_copies:
        c.wait()

    def project(b, carry):
        x_copy(b + 1).wait()

        @pl.when(b == 1)
        def _():
            for k in range(3, NB):
                x_copy(k).start()

        projections(b, False)
        return carry

    lax.fori_loop(0, NB - 1, project, 0)
    for c in w_copies(1, 0):
        c.start()
    projections(NB - 1, True)

    bound2 = jnp.max(norm_s[0]) * jnp.max(norm_s[1])
    v_max = jnp.max(norm_s[2])
    safe = (bound2 <= 50.0 ** 2) & (v_max <= 2.0 ** 40) & (v_max >= 2.0 ** -30)

    @pl.when(jnp.logical_not(safe))
    def _():
        def attend_with_max(i, carry):
            blk, h = i // H, i % H
            q = unpack(qt_s[blk, pl.ds(pl.multiple_of(h * (DH // 2), DH // 2), DH // 2), :])
            s = mm(unpack(k_s[...])[:, 0:DH], q)
            p = jnp.exp2(s - jnp.max(s, axis=0, keepdims=True))
            vt = jnp.concatenate([unpack(vt_s[c]) for c in range(NC)], axis=1)
            o = mm(vt, p.astype(BF16)) / jnp.sum(p, axis=0, keepdims=True)
            for t in range(TQ // 128):
                @pl.when(blk % (TQ // 128) == t)
                def _():
                    ot_s[blk // (TQ // 128), pl.ds(pl.multiple_of(h * DH, DH), DH), tile(t)] = o
            return carry

        lax.fori_loop(0, S // 128 * H, attend_with_max, 0)

    def step(b, j):
        last = j == NJ - 1
        n_ffn, groups = FFN_TILES[j], GROUPS[j]
        units = HEADS[j] // HU
        early = groups - 1 if last else groups
        r0 = pl.multiple_of(b * TQ, TQ)
        z_store = pl.multiple_of(zero_s[0], 8)
        z_load = pl.multiple_of(zero_s[1], 8)
        z = zero_s[2]

        def fence(v):
            fence_s[pl.ds(z_store, 8), 0:128] = v

        latest = [None]
        pin_latest = lambda ref: pin(ref, latest[0])
        side = iter(()) if last else prepare_weights(j + 1, b, pin_latest)
        n_side = 0 if last else 7 * (KG // NB // 16 * (FFN_TILES[j + 1] // 2) + GROUPS[j + 1] * (KG // 128))
        side_time = units * S + NPROD * (KG // 128) * (MB * groups // 4) - 300
        queue = []
        state = dict(time=0, pieces=0, credit=0.0, gap=96, hold=False)

        def pump(n):
            while n and queue and not state["hold"]:
                v = next(queue[0], None)
                if v is None:
                    queue.pop(0)
                else:
                    fence(pltpu.bitcast(v, F32))
                    n -= 1

        def tick(v, cycles, with_side):
            state["time"] += cycles * with_side
            fence(v)
            latest[0] = v
            while state["pieces"] < min(n_side, n_side * state["time"] // side_time):
                fence(pltpu.bitcast(next(side)(z), F32))
                state["pieces"] += 1
            state["credit"] += cycles / state["gap"]
            pump(int(state["credit"]))
            state["credit"] -= int(state["credit"])

        def left_operands(p):
            dst, t = (ha_s, p) if p < early else (hb_s, p - early)
            for i0 in range(0, MB, 16):
                load = lambda r, k: hf_s[pl.ds(z_load + r * MB + i0, 16), tile(p * G + k)]
                for i, v in operands(LEFT, G, load, lambda: pin_latest(hf_s)):
                    dst[i, i0 // 2:i0 // 2 + 8, tile(t)] = pack(v)
                    if i % 7 == 6:
                        yield dst[i + z, i0 // 2:i0 // 2 + 8, tile(t)]

        filled = [0] * groups

        def put(t, row, v):
            hf_s[pl.ds(z_store + row, v.shape[0]), tile(t)] = v
            filled[t // G] += v.shape[0]
            if filled[t // G] == G * TQ:
                queue.append(left_operands(t // G))

        def put_attention(t):
            for half in range(TQ // 128):
                put(n_ffn + t, half * 128,
                    ot_s[b + z, tile(OUT0[j] + t), tile(half)].T * g_s[pl.ds(r0 + half * 128, 128), :])

        def gate_up(t):
            blocks = {}

            def emit(r, c, v):
                blocks[r, c] = v
                k = c % 2
                if (r, k) in blocks and (r, 2 + k) in blocks:
                    put(t * 2 + k, r * MB,
                        jnp.maximum(blocks.pop((r, k)), 0.0) * blocks.pop((r, 2 + k))
                        * (1.0 - g_s[pl.ds(r0 + r * MB, MB), :]))

            for v in strassen(G, lambda i: mm(unpack(xa_s[b, i]), unpack(wgu[j % 2][i, :, tile(t)])), emit):
                tick(v[MB - 8:], MB * (KG // 128) // 4, False)

        def down(n, lo, hi):
            def emit(r, c, v):
                cols = tile(c * KG // 128 + n)
                if sum(GROUPS[:j]) + lo > 0:
                    v = acc_s[pl.ds(r0 + r * MB, MB), cols] + v
                if last and hi == groups:
                    out_s[b % 2, r * MB:(r + 1) * MB, cols] = v.astype(out_s.dtype)
                else:
                    acc_s[pl.ds(r0 + r * MB, MB), cols] = v

            def product(i):
                lhs = jnp.concatenate([ha_s[i + z, :, 0:early * 128]] * (lo == 0)
                                      + [hb_s[i + z, :, 0:(hi - early) * 128]] * (hi > early), axis=1)
                return mm(unpack(lhs), unpack(wdn[j % 2][i, lo * 64:hi * 64, tile(n)]))

            for v in strassen(G, product, emit):
                tick(v[MB - 8:], MB * (hi - lo) // 4, True)
                yield

        steps = [(u, c) for u in range(units) for c in range(NC)]
        run = {}
        probs = {}

        def scores(u, c):
            k = jnp.concatenate([k_s[r // 2:r // 2 + 8, :]
                                 for r in range((c + 1) * KC - 16, c * KC - 1, -16)], axis=0)
            h = HEAD0[j] + u * HU
            q = jnp.concatenate(
                [unpack(qt_s[b * (TQ // 128) + t, (h + i) * (DH // 2):(h + i + 1) * (DH // 2), :])
                 for i in range(HU) for t in range(TQ // 128)], axis=1)
            s = mm(unpack(k)[:, 0:DH], q)
            for i in range(32, KC + 1, 32):
                tick(s[i - 8:i, 0:128], 32, True)
            p = jnp.exp2(jnp.concatenate([s[i:i + 16] for i in range(KC - 16, -1, -16)], axis=0))
            run["sum"] = fold8(p, jnp.add, run["sum"] if c else None, reverse=True)
            probs[u, c] = (p.astype(BF16), run["sum"])
            fence_s[pl.ds(z_store + 8, 8), :] = run["sum"]

        def attend(u, c):
            p, total = probs.pop((u, c))
            d = mm(unpack(vt_s[c]), p)
            run["out"] = run["out"] + d if c else d
            if c == NC - 1:
                o = run["out"] * (1.0 / jnp.sum(total, axis=0, keepdims=True))
                for i in range(HU):
                    rows = slice((HEAD0[j] + u * HU + i) * DH, (HEAD0[j] + u * HU + i + 1) * DH)
                    ot_s[b, rows, :] = jnp.where(safe, o[:, i * TQ:(i + 1) * TQ], ot_s[b, rows, :])

        if not last:
            for c in w_copies(j + 1, b + 1):
                c.start()
        ready = [t for t in range(OUT_TILES[j]) if (OUT0[j] + t + 1) * 128 <= HEAD0[j] * DH]
        head = 1 if n_ffn else 0
        for i in range(head):
            scores(*steps[i])
        for t in range(n_ffn // 2):
            gate_up(t)
            if t == 0:
                for k in ready:
                    put_attention(k)
        parts = []
        if groups:
            parts.append(down(0, 0, early))
            if early < groups:
                parts.append(down(0, early, groups))
            parts += [down(n, 0, groups) for n in range(1, KG // 128)]
        done = 0
        for i in range(len(steps)):
            if i >= head:
                scores(*steps[i])
            while done + 2 <= i < len(steps) - (0 if groups else 4):
                attend(*steps[done])
                done += 1
        for i in range(done, len(steps)):
            if groups:
                pump(NPROD * groups)
                next(parts[0])
                next(parts[0])
            attend(*steps[i])
        state["gap"] = 56
        for t in range(OUT_TILES[j]):
            if t not in ready:
                next(parts[0])
                next(parts[0])
                put_attention(t)
        if len(ready) < OUT_TILES[j]:
            state["hold"] = True
            next(parts[0])
            next(parts[0])
            state["hold"] = False
        for part in parts:
            drain(part)
            pump(NPROD * groups)
        drain(side)

    for j in range(NJ):
        def body(b, carry):
            if j < NJ - 1:
                for c in w_copies(j + 1, b):
                    c.wait()
            else:
                @pl.when(b >= 2)
                def _():
                    o_copy(b - 2).wait()
            step(b, j)
            if j == NJ - 1:
                o_copy(b).start()
            return carry

        if j + 2 < NJ:
            for c in w_copies(j + 2, 0):
                c.start()
        lax.fori_loop(0, NB, body, 0)
        if j + 1 < NJ:
            for c in w_copies(j + 1, NB):
                c.wait()
    o_copy(NB - 2).wait()
    o_copy(NB - 1).wait()


@jax.jit
def pallas_gated_mix__grouped_kv_mqa__glu_gated_reglu__prompt_kernel(
    A_x: jax.Array,
    A_wq: jax.Array,
    A_wk: jax.Array,
    A_wv: jax.Array,
    A_wo: jax.Array,
    B_x: jax.Array,
    B_W_gate: jax.Array,
    B_W_up: jax.Array,
    B_W_down: jax.Array,
    gate_w: jax.Array,
):
    del B_x
    assert A_x.shape == (1, S, D) and B_W_gate.shape == (D, F) and A_wk.shape == (D, DH)
    hbm = pl.BlockSpec(memory_space=pl.ANY)
    out = pl.pallas_call(
        kernel,
        in_specs=[hbm] * 9,
        out_specs=hbm,
        out_shape=jax.ShapeDtypeStruct((S, D), A_x.dtype),
        scratch_shapes=[
            pltpu.VMEM((S + 32, D), BF16),
            pltpu.VMEM((D, D), BF16),
            pltpu.VMEM((DH, D), BF16),
            pltpu.VMEM((DH, D), BF16),
            pltpu.VMEM((64, 128), BF16),
            pltpu.VMEM((2, 128, 128), F32),
            pltpu.VMEM((4 * G + 1, KG // NB, FM * 128), BF16),
            pltpu.VMEM((4 * G + 1, KG // NB, FM * 128), BF16),
            pltpu.VMEM((4 * GM * G + 1, 16, D), BF16),
            pltpu.VMEM((NB, NPROD, MB // 2, KG), U32),
            pltpu.VMEM((NPROD, KG // 2, FM // 2 * 128), U32),
            pltpu.VMEM((NPROD, KG // 2, FM // 2 * 128), U32),
            pltpu.VMEM((NPROD, max(GROUPS[0::2]) * 64, KG), U32),
            pltpu.VMEM((NPROD, max(GROUPS[1::2]) * 64, KG), U32),
            pltpu.VMEM((S // 2, 128), U32),
            pltpu.VMEM((S // 128, DH // 2, 128), U32),
            pltpu.VMEM((S, 128), F32),
            pltpu.VMEM((S // 128 + 1, D // 2, 128), U32),
            pltpu.VMEM((NB, D, TQ), F32),
            pltpu.VMEM((24, 512), F32),
            pltpu.VMEM((4, 8, TQ), F32),
            pltpu.VMEM((NPROD, MB // 2, max(GROUPS[:-1]) * 128), U32),
            pltpu.VMEM((NPROD, MB // 2, 128), U32),
            pltpu.VMEM((TQ + 32, GM * G * 128), F32),
            pltpu.VMEM((S, D), F32),
            pltpu.VMEM((2, TQ, D), A_x.dtype),
            pltpu.SMEM((4,), jnp.int32),
            pltpu.SemaphoreType.DMA((NB,)),
            pltpu.SemaphoreType.DMA((NQ * G,)),
            pltpu.SemaphoreType.DMA((3,)),
            pltpu.SemaphoreType.DMA((16,)),
            pltpu.SemaphoreType.DMA((2,)),
        ],
        compiler_params=pltpu.CompilerParams(vmem_limit_bytes=127 * 2**20),
        name="gated_mix",
    )(A_x.reshape(S, D), A_wq, A_wk.T, A_wv.T, A_wo.reshape(D // 128, 128, D),
      B_W_gate.reshape(G, KG, F), B_W_up.reshape(G, KG, F), B_W_down.reshape(F // 128, 128, D),
      gate_w.reshape(D // 128, 128))
    return out.reshape(A_x.shape)
```

```python
import functools

import jax
import jax.numpy as jnp
from jax import lax
from jax.experimental import pallas as pl
from jax.experimental.pallas import tpu as pltpu

F32 = jnp.float32
BF16 = jnp.bfloat16
U32 = jnp.uint32
LOG2E = 1.4426950408889634

S, D, F, H = 2048, 1024, 3584, 32
DH = D // H
TQ = 256
NB = S // TQ
KC = 128
NC = S // KC
HU = 512 // TQ
G = 4
NPROD = 49
MB = TQ // G
KG = D // G

HEADS = (10, 8, 14)
FFN_GROUPS = (0, 4, 3)
OUT_GROUPS = (0, 0, 2)
NJ = len(HEADS)
HEAD0 = [sum(HEADS[:j]) for j in range(NJ)]
FFN0 = [sum(FFN_GROUPS[:j]) for j in range(NJ)]
GROUPS = [FFN_GROUPS[j] + OUT_GROUPS[j] for j in range(NJ)]
FM, GM = max(FFN_GROUPS), max(GROUPS)
NQ = 4
QR = KG // NQ

ADD, SUB = jnp.add, jnp.subtract
LEFT = ((SUB, 0, 3), (SUB, 2, 3), (None, 0, 0), (None, 3, 3), (SUB, 1, 0), (SUB, 2, 0), (SUB, 1, 3))
RIGHT = ((SUB, 0, 3), (None, 0, 0), (ADD, 1, 3), (ADD, 2, 0), (None, 3, 3), (ADD, 0, 1), (ADD, 2, 3))
USES = (((0, 1), (3, 1)), ((2, 1), (3, -1)), ((1, 1), (3, 1)), ((0, 1), (2, 1)), ((0, -1), (1, 1)),
        ((3, 1),), ((0, 1),))
ORDER = (6, 4, 3, 2, 1, 0, 5)
SWAP = (2, 4, 5, 6)


def mm(a, b):
    return jnp.dot(a, b, preferred_element_type=F32)


def pack(x):
    return pltpu.bitcast(x.astype(BF16), U32)


def unpack(x):
    return pltpu.bitcast(x, BF16)


def tile(i):
    return slice(i * 128, (i + 1) * 128)


def fold8(x, op, r=None, reverse=False):
    groups = range(x.shape[0] // 8)
    for i in reversed(groups) if reverse else groups:
        v = x[8 * i:8 * i + 8]
        r = v if r is None else op(r, v)
    return r


def operands(table, n, load, before=None):
    h = n // 2
    for i, (op, x, y) in enumerate(table):
        if before:
            before()
        at = lambda q, r, c: load(q // 2 * h + r, q % 2 * h + c)
        g = [[op(at(x, r, c).astype(F32), at(y, r, c).astype(F32)) if op else at(x, r, c)
              for c in range(h)] for r in range(h)]
        if h == 1:
            yield i, g[0][0]
        else:
            flip = int(table is RIGHT and i in SWAP)
            for k, v in operands(table, h, lambda r, c: g[r][c ^ flip]):
                yield i * 7 + k, v


def strassen(n, product, emit, base=0):
    if n == 1:
        m = product(base)
        emit(0, 0, m)
        yield m
        return
    h = n // 2
    acc = {}
    left = [4, 2, 2, 4]
    for r in ORDER:
        for q, _ in USES[r]:
            left[q] -= 1

        def sink(i, k, m, r=r):
            if h > 1 and r in SWAP:
                k ^= 1
            for q, sign in USES[r]:
                key = (q // 2 * h + i, q % 2 * h + k)
                if key in acc:
                    v = acc.pop(key) + m if sign > 0 else acc.pop(key) - m
                else:
                    assert sign > 0
                    v = m
                if left[q]:
                    acc[key] = v
                else:
                    emit(key[0], key[1], v)

        yield from strassen(h, product, sink, base * 7 + r)


def drain(gen):
    for _ in gen:
        pass


def kernel(x_hbm, wq_hbm, wkt_hbm, wvt_hbm, wo_hbm, wg_hbm, wu_hbm, wd_hbm, gw_hbm, o_hbm,
           wg_s, wu_s, wd_s, xa_s, wgu_a, wgu_b, wdn_a, wdn_b,
           k_s, vt_s, g_s, mix_s, qt_s, ot_s, fence_s, norm_s, zero_s,
           x_sem, q_sem, k_sem, w_sem, o_sem):
    wgu = (wgu_a, wgu_b)
    wdn = (wdn_a, wdn_b)
    wqc_s = wgu_a

    def w_slot(j, b):
        return jnp.where(b == 0, 2 + j % 2, b % 2)

    def w_copies(j, b):
        nf, no, slot, r = FFN_GROUPS[j] * G, OUT_GROUPS[j] * G, w_slot(j, b), KG // NB
        b = jnp.minimum(b, NB - 1)
        rows = pl.ds(pl.multiple_of(b * r, r), r)
        cols = pl.ds(FFN0[j] * G * 128, nf * 128)
        drows = pl.ds(pl.multiple_of(b * 16, 16), 16)
        copies = [
            pltpu.make_async_copy(wg_hbm.at[:, rows, cols],
                                  wg_s.at[pl.ds(slot * G, G), :, pl.ds(0, nf * 128)], w_sem.at[4 * slot]),
            pltpu.make_async_copy(wu_hbm.at[:, rows, cols],
                                  wu_s.at[pl.ds(slot * G, G), :, pl.ds(0, nf * 128)], w_sem.at[4 * slot + 1]),
            pltpu.make_async_copy(wd_hbm.at[pl.ds(FFN0[j] * G, nf), drows],
                                  wd_s.at[pl.ds(slot * GM * G, nf)], w_sem.at[4 * slot + 2])]
        if no:
            copies.append(pltpu.make_async_copy(wo_hbm.at[:, drows], wd_s.at[pl.ds(slot * GM * G + nf, no)],
                                                w_sem.at[4 * slot + 3]))
        return copies

    def pin(ref, v):
        if len(ref.shape) == 3:
            ref[zero_s[0] + ref.shape[0] - 1, 0:8, 0:128] = v.astype(ref.dtype)
        else:
            ref[pl.ds(pl.multiple_of(zero_s[0], 8) + ref.shape[0] - 32, 8), 0:128] = v.astype(ref.dtype)

    def operand_pieces(table, load, store, before):
        for i, v in operands(table, G, load, before):
            reread = store(i, pack(v))
            if i % 7 == 6:
                yield reread

    def right_store(dst, row, t):
        def store(i, v):
            dst[i, pl.ds(row, 8), tile(t)] = v
            return lambda z: dst[i + z, pl.ds(row, 8), tile(t)]
        return store

    def prepare_weights(j, b, pin_latest):
        r = KG // NB
        slot = w_slot(j, b)
        p0 = pl.multiple_of(b * (r // 2), r // 2)
        for i0 in range(0, r, 16):
            for t in range(2 * FFN_GROUPS[j]):
                src = (wg_s, wu_s)[t % 2]
                load = lambda k, c: src[slot * G + k, i0:i0 + 16, tile(t // 2 * G + (c ^ t % 2 * 2))]
                yield from operand_pieces(RIGHT, load, right_store(wgu[j % 2], p0 + i0 // 2, t),
                                          lambda: pin_latest(src))
        p0 = pl.multiple_of(b * 8, 8)
        for p in range(GROUPS[j]):
            for n in range(KG // 128):
                load = lambda k, c: wd_s[slot * GM * G + p * G + k, :, tile(c * KG // 128 + n)]
                yield from operand_pieces(RIGHT, load, right_store(wdn[j % 2], p * 64 + p0, n),
                                          lambda: pin_latest(wd_s))

    def inputs(x_s, xn_s, wq_s, wkt_s, wvt_s, gw_s, qh_s):
        def x_copy(b):
            return pltpu.make_async_copy(x_hbm.at[pl.ds(b * TQ, TQ)], x_s.at[pl.ds(b * TQ, TQ)], x_sem.at[b])

        def q_copies(p):
            return [pltpu.make_async_copy(wq_hbm.at[pl.ds(k * KG + p * QR, QR)],
                                          wq_s.at[pl.ds(k * KG + p * QR, QR)], q_sem.at[p * G + k])
                    for k in range(G)]

        kv_copies = [pltpu.make_async_copy(wkt_hbm, wkt_s, k_sem.at[0]),
                     pltpu.make_async_copy(wvt_hbm, wvt_s, k_sem.at[1]),
                     pltpu.make_async_copy(gw_hbm, gw_s.at[pl.ds(0, 8)], k_sem.at[2])]

        def prepare_wq(p, carry):
            for c in q_copies(p):
                c.wait()

            @pl.when(p + 2 < NQ)
            def _():
                for c in q_copies(p + 2):
                    c.start()

            @pl.when(p + 2 == NQ)
            def _():
                x_copy(0).start()

            @pl.when(p + 1 == NQ)
            def _():
                x_copy(1).start()
                for c in kv_copies:
                    c.start()

            r0 = pl.multiple_of(p * QR, QR)
            p0 = pl.multiple_of(p * (QR // 2), QR // 2)
            for i0 in range(0, QR, 16):
                for n in range(KG // 128):
                    load = lambda k, c: wq_s[pl.ds(r0 + k * KG + i0, 16), tile(c * KG // 128 + n)]
                    drain(operand_pieces(RIGHT, load, right_store(wqc_s, p0 + i0 // 2, n), None))
            return carry

        def prepare_x(b, src, r0, before):
            for n in range(KG // 128):
                for i0 in range(0, MB, 16):
                    load = lambda r, c: src[pl.ds(r0 + r * MB + i0, 16), tile(c * KG // 128 + n)]

                    def store(i, v):
                        xa_s[b, i, i0 // 2:i0 // 2 + 8, tile(n)] = v
                        return lambda z: xa_s[b, i + z, i0 // 2:i0 // 2 + 8, tile(n)]
                    yield from operand_pieces(LEFT, load, store, before)

        def keys_values(b):
            r0 = pl.multiple_of(b * TQ, TQ)
            gw = gw_s[0:8, :].astype(F32)
            gw = jnp.concatenate([jnp.broadcast_to(gw[i:i + 1], (16, 128)) for i in range(D // 128)], axis=1)
            w = jnp.concatenate([wkt_s[...], wvt_s[...], gw.astype(BF16)], axis=0)
            kvz = lax.dot_general(w, x_s[pl.ds(r0, TQ), :], (((1,), (1,)), ((), ())),
                                  preferred_element_type=F32)
            for i in range(TQ // 128):
                vt_s[2 * b + i] = pack(kvz[DH:2 * DH, tile(i)])
            kt = kvz[0:DH] * (DH ** -0.5 * LOG2E)
            norm_s[1] = jnp.maximum(norm_s[1], jnp.sum(kt * kt, axis=0, keepdims=True))
            norm_s[2] = fold8(jnp.abs(kvz[DH:2 * DH]), jnp.maximum, norm_s[2])
            kt = jnp.concatenate([kt, jnp.zeros((128 - DH, TQ), F32)], axis=0)
            k_s[pl.ds(pl.multiple_of(b * (TQ // 2), TQ // 2), TQ // 2), :] = pltpu.bitcast(kt.astype(BF16).T, U32)
            g = jax.nn.sigmoid(kvz[2 * DH:2 * DH + 1])
            g = jnp.broadcast_to(g, (128, TQ)).T
            g_s[pl.ds(r0, TQ), :] = g
            mix_s[pl.ds(r0, TQ), :] = 1.0 - g

        def projections(b, last):
            latest = [None]
            side = iter(()) if last else prepare_x(
                b + 1, x_s, pl.multiple_of((b + 1) * TQ, TQ), lambda: pin(x_s, latest[0]))
            n_side = 0 if last else KG // 128 * (MB // 16) * 7
            norm = [norm_s[0, :, 0:128]]
            sizes = [[], []]

            def put_q(row, half, t, q):
                qt = q.astype(BF16).T
                qt_s[row, t * 64:(t + 1) * 64, :] = pltpu.bitcast(qt, U32)
                qf = qt.astype(F32)
                ot_s[row // 2, tile(t), tile(half)] = qf
                q2 = qf * qf
                for i in range(128 // DH):
                    n2 = fold8(q2[i * DH:(i + 1) * DH], jnp.add)
                    norm[0] = jnp.maximum(norm[0], n2)
                    if t % 2 == 0:
                        sizes[half].append(n2)
                norm_s[0, :, 0:128] = norm[0]

            if last:
                keys_values(b)
            for i in range(2):
                put_q(jnp.maximum(2 * b - 1, 1), 1, 5 + 2 * i, qh_s[i])
            products = pieces = 0
            for n in range(KG // 128):
                blocks = {}

                def emit(r, c, v):
                    blocks[r, c] = v
                    top = r // 2 * 2
                    if (top, c) in blocks and (top + 1, c) in blocks:
                        q = jnp.concatenate([blocks.pop((top, c)), blocks.pop((top + 1, c))], axis=0)
                        if not last and n == 1 and r >= 2 and c >= 2:
                            qh_s[c - 2] = q
                        else:
                            put_q(2 * b + r // 2, r // 2, c * KG // 128 + n, q)

                for v in strassen(G, lambda i: mm(unpack(xa_s[b, i]), unpack(wqc_s[i, :, tile(n)])), emit):
                    latest[0] = v[0:8]
                    products += 1
                    if not last and products == 2:
                        keys_values(b)
                    while pieces < min(n_side, n_side * (products - 2) // (NPROD * (KG // 128) - 14)):
                        qt_s[S // 128 + zero_s[0], 0:8, :] = next(side)(zero_s[2])
                        pieces += 1
                if n == 0:
                    size = jnp.concatenate([functools.reduce(jnp.add, v) for v in sizes], axis=1)
                    size = jnp.sum(size, axis=0, keepdims=True)
                    norm_s[3] = jnp.maximum(norm_s[3], size)
                    norm_s[4] = jnp.minimum(norm_s[4], size)

        for c in q_copies(0):
            c.start()
        for i in range(4):
            zero_s[i] = 0
        norm_s[0:4] = jnp.zeros((4, 8, TQ), F32)
        norm_s[4] = jnp.full((8, TQ), jnp.inf, F32)
        qh_s[...] = jnp.zeros(qh_s.shape, F32)
        for c in q_copies(1):
            c.start()
        lax.fori_loop(0, NQ, prepare_wq, 0)
        x_copy(0).wait()
        drain(prepare_x(0, x_s, 0, None))
        x_copy(2).start()
        for c in kv_copies:
            c.wait()

        def project(b, carry):
            x_copy(b + 1).wait()

            @pl.when(b == 1)
            def _():
                for k in range(3, NB):
                    x_copy(k).start()

            projections(b, False)
            return carry

        lax.fori_loop(0, NB - 1, project, 0)
        for c in w_copies(1, 0):
            c.start()
        projections(NB - 1, True)

        bound2 = jnp.max(jnp.sum(norm_s[0], axis=0, keepdims=True)) * jnp.max(norm_s[1])
        v_max = jnp.max(norm_s[2])
        safe = (bound2 <= 50.0 ** 2) & (v_max <= 2.0 ** 40) & (v_max >= 2.0 ** -30)
        safe &= jnp.max(norm_s[3]) <= 16.0 * jnp.min(norm_s[4])

        @pl.when(jnp.logical_not(safe))
        def _():
            def equilibrate(b, carry):
                rows = pl.ds(pl.multiple_of(b * TQ, TQ), TQ)
                x = x_s[rows, :].astype(F32)
                size = jnp.broadcast_to(jnp.sum(jnp.abs(x), axis=1, keepdims=True) * (1.0 / D), (TQ, 128))
                power = pltpu.bitcast(jnp.clip(size, 2.0 ** -40, 2.0 ** 40), jnp.int32) >> 23 << 23
                scale = pltpu.bitcast(power, F32)
                xn_s[...] = x * jnp.concatenate([pltpu.bitcast((254 << 23) - power, F32)] * (D // 128), axis=1)
                mix_s[rows, :] = mix_s[rows, :] * (scale * scale)
                drain(prepare_x(b, xn_s, 0, None))
                return carry

            lax.fori_loop(0, NB, equilibrate, 0)

            def plain_queries(i, carry):
                blk, t = i // G, i % G
                x = x_s[pl.ds(pl.multiple_of(blk * 128, 128), 128), :]
                q = mm(x, wq_s[:, pl.ds(pl.multiple_of(t * KG, KG), KG)]).astype(BF16).T
                qt_s[blk, pl.ds(pl.multiple_of(t * (KG // 2), KG // 2), KG // 2), :] = pltpu.bitcast(q, U32)
                return carry

            lax.fori_loop(0, S // 128 * G, plain_queries, 0)

            def attend_with_max(i, carry):
                blk, h = i // H, i % H
                q = unpack(qt_s[blk, pl.ds(pl.multiple_of(h * (DH // 2), DH // 2), DH // 2), :])
                s = mm(unpack(k_s[...])[:, 0:DH], q)
                p = jnp.exp2(s - jnp.max(s, axis=0, keepdims=True))
                vt = jnp.concatenate([unpack(vt_s[c]) for c in range(NC)], axis=1)
                o = mm(vt, p.astype(BF16)) / jnp.sum(p, axis=0, keepdims=True)
                for t in range(TQ // 128):
                    @pl.when(blk % (TQ // 128) == t)
                    def _():
                        ot_s[blk // (TQ // 128), pl.ds(pl.multiple_of(h * DH, DH), DH), tile(t)] = o
                return carry

            lax.fori_loop(0, S // 128 * H, attend_with_max, 0)
        return safe

    safe = pl.run_scoped(
        inputs,
        pltpu.VMEM((S + 32, D), BF16),
        pltpu.VMEM((TQ, D), F32),
        pltpu.VMEM((D, D), BF16),
        pltpu.VMEM((DH, D), BF16),
        pltpu.VMEM((DH, D), BF16),
        pltpu.VMEM((64, 128), BF16),
        pltpu.VMEM((2, 128, 128), F32))

    def stages(ha_s, hb_s, hf_s, gate_s, acc_s, out_s):
        def o_copy(b):
            return pltpu.make_async_copy(out_s.at[b % 2], o_hbm.at[pl.ds(b * TQ, TQ)], o_sem.at[b % 2])

        def step(b, j):
            last = j == NJ - 1
            n_ffn, groups = FFN_GROUPS[j], GROUPS[j]
            units = HEADS[j] // HU
            r0 = pl.multiple_of(b * TQ, TQ)
            z_store = pl.multiple_of(zero_s[0], 8)
            z_load = pl.multiple_of(zero_s[1], 8)
            z = zero_s[2]

            def fence(v):
                fence_s[pl.ds(z_store, 8), 0:128] = v

            latest = [None]
            pin_latest = lambda ref: pin(ref, latest[0])
            side = iter(()) if last else prepare_weights(j + 1, b, pin_latest)
            n_side = 0 if last else 7 * (KG // NB // 16 * 2 * FFN_GROUPS[j + 1] + GROUPS[j + 1] * (KG // 128))
            side_time = units * S + NPROD * (KG // 128) * (MB * groups // 4) - 300
            queue = []
            state = dict(time=0, pieces=0, credit=0.0, hold=False)

            def pump(n):
                while n and queue and not state["hold"]:
                    v = next(queue[0], None)
                    if v is None:
                        queue.pop(0)
                    else:
                        fence(pltpu.bitcast(v, F32))
                        n -= 1

            def tick(v, cycles, with_side):
                state["time"] += cycles * with_side
                fence(v)
                latest[0] = v
                while state["pieces"] < min(n_side, n_side * state["time"] // side_time):
                    fence(pltpu.bitcast(next(side)(z), F32))
                    state["pieces"] += 1
                state["credit"] += cycles / 72
                pump(int(state["credit"]))
                state["credit"] -= int(state["credit"])

            def left_operands(p):
                dst, t = (ha_s, p) if p < n_ffn else (hb_s, p - n_ffn)
                for i0 in range(0, MB, 16):
                    load = lambda r, k: hf_s[pl.ds(z_load + r * MB + i0, 16), tile(p * G + k)]
                    for i, v in operands(LEFT, G, load, lambda: pin_latest(hf_s)):
                        dst[i, i0 // 2:i0 // 2 + 8, tile(t)] = pack(v)
                        if i % 7 == 6:
                            yield dst[i + z, i0 // 2:i0 // 2 + 8, tile(t)]

            filled = [0] * groups

            def put(t, row, v):
                hf_s[pl.ds(z_store + row, v.shape[0]), tile(t)] = v
                filled[t // G] += v.shape[0]
                if filled[t // G] == G * TQ:
                    queue.append(left_operands(t // G))

            def put_attention(t):
                for half in range(TQ // 128):
                    put(n_ffn * G + t, half * 128, ot_s[b + z, tile(t), tile(half)].T)

            def gate_up(t):
                def emit(r, c, v):
                    if t % 2 == 0:
                        gate_s[pl.ds(z_store + r * MB, MB), tile(c)] = jnp.maximum(v, 0.0)
                    else:
                        c ^= 2
                        put(t // 2 * G + c, r * MB, gate_s[pl.ds(z_load + r * MB, MB), tile(c)] * v)

                for v in strassen(G, lambda i: mm(unpack(xa_s[b, i]), unpack(wgu[j % 2][i, :, tile(t)])), emit):
                    tick(v[MB - 8:], MB * (KG // 128) // 4, False)

            def project_out(n, hidden):
                src, lo, hi = (ha_s, 0, n_ffn) if hidden else (hb_s, n_ffn, groups)

                def emit(r, c, v):
                    rows, cols = pl.ds(r0 + r * MB, MB), tile(c * KG // 128 + n)
                    v = v * (mix_s if hidden else g_s)[rows, :]
                    if sum(GROUPS[:j]) + lo > 0:
                        v = acc_s[rows, cols] + v
                    if last and hi == groups:
                        out_s[b % 2, r * MB:(r + 1) * MB, cols] = v.astype(out_s.dtype)
                    else:
                        acc_s[rows, cols] = v

                product = lambda i: mm(unpack(src[i + z, :, 0:(hi - lo) * 128]),
                                       unpack(wdn[j % 2][i, lo * 64:hi * 64, tile(n)]))
                for v in strassen(G, product, emit):
                    tick(v[MB - 8:], MB * (hi - lo) // 4, True)
                    yield

            steps = [(u, c) for u in range(units) for c in range(NC)]
            run = {}
            probs = {}

            def scores(u, c):
                k = jnp.concatenate([k_s[r // 2:r // 2 + 8, :]
                                     for r in range((c + 1) * KC - 16, c * KC - 1, -16)], axis=0)
                h = HEAD0[j] + u * HU
                q = jnp.concatenate(
                    [unpack(qt_s[b * (TQ // 128) + t, (h + i) * (DH // 2):(h + i + 1) * (DH // 2), :])
                     for i in range(HU) for t in range(TQ // 128)], axis=1)
                s = mm(unpack(k)[:, 0:DH], q)
                for i in range(32, KC + 1, 32):
                    tick(s[i - 8:i, 0:128], 32, True)
                p = jnp.exp2(jnp.concatenate([s[i:i + 16] for i in range(KC - 16, -1, -16)], axis=0))
                run["sum"] = fold8(p, jnp.add, run["sum"] if c else None, reverse=True)
                probs[u, c] = (p.astype(BF16), run["sum"])
                fence_s[pl.ds(z_store + 8, 8), :] = run["sum"]

            def attend(u, c):
                p, total = probs.pop((u, c))
                d = mm(unpack(vt_s[c]), p)
                run["out"] = run["out"] + d if c else d
                if c == NC - 1:
                    o = run["out"] * (1.0 / jnp.sum(total, axis=0, keepdims=True))
                    for i in range(HU):
                        rows = slice((HEAD0[j] + u * HU + i) * DH, (HEAD0[j] + u * HU + i + 1) * DH)
                        ot_s[b, rows, :] = jnp.where(safe, o[:, i * TQ:(i + 1) * TQ], ot_s[b, rows, :])

            if not last:
                for c in w_copies(j + 1, b + 1):
                    c.start()
            out_tiles = range(OUT_GROUPS[j] * G)
            ready = [t for t in out_tiles if (t + 1) * 128 <= HEAD0[j] * DH]
            head = 1 if n_ffn else 0
            for i in range(head):
                scores(*steps[i])
            for t in range(2 * n_ffn):
                gate_up(t)
                for k in ready[t::2 * n_ffn]:
                    put_attention(k)
            parts = [project_out(n, hidden) for hidden, count in ((True, n_ffn), (False, OUT_GROUPS[j]))
                     for n in range(KG // 128) if count]
            done = 0
            for i in range(len(steps)):
                if i >= head:
                    scores(*steps[i])
                while done + 2 <= i < len(steps) - (0 if groups else 4):
                    attend(*steps[done])
                    done += 1
            for i in range(done, len(steps)):
                if groups:
                    pump(NPROD * groups)
                    for _ in range(2):
                        next(parts[0])
                attend(*steps[i])
            for t in out_tiles:
                if t not in ready:
                    for _ in range(2):
                        next(parts[0])
                    put_attention(t)
            if len(ready) < len(out_tiles):
                state["hold"] = True
                next(parts[0])
                next(parts[0])
                state["hold"] = False
            for i, part in enumerate(parts):
                if i == KG // 128:
                    pump(NPROD * groups)
                drain(part)
            drain(side)

        for j in range(NJ):
            def body(b, carry):
                if j == NJ - 1:
                    @pl.when(b >= 2)
                    def _():
                        o_copy(b - 2).wait()
                step(b, j)
                if j == NJ - 1:
                    o_copy(b).start()
                else:
                    for c in w_copies(j + 1, b + 1):
                        c.wait()
                return carry

            if j + 2 < NJ:
                for c in w_copies(j + 2, 0):
                    c.start()
            if j + 1 < NJ:
                for c in w_copies(j + 1, 0):
                    c.wait()
            lax.fori_loop(0, NB, body, 0)
        o_copy(NB - 2).wait()
        o_copy(NB - 1).wait()

    pl.run_scoped(
        stages,
        pltpu.VMEM((NPROD, MB // 2, FM * 128), U32),
        pltpu.VMEM((NPROD, MB // 2, max(OUT_GROUPS) * 128), U32),
        pltpu.VMEM((TQ + 32, GM * G * 128), F32),
        pltpu.VMEM((TQ + 8, G * 128), F32),
        pltpu.VMEM((S, D), F32),
        pltpu.VMEM((2, TQ, D), o_hbm.dtype))


@jax.jit
def pallas_gated_mix__grouped_kv_mqa__glu_gated_reglu__prompt_kernel(
    A_x: jax.Array,
    A_wq: jax.Array,
    A_wk: jax.Array,
    A_wv: jax.Array,
    A_wo: jax.Array,
    B_x: jax.Array,
    B_W_gate: jax.Array,
    B_W_up: jax.Array,
    B_W_down: jax.Array,
    gate_w: jax.Array,
):
    del B_x
    assert A_x.shape == (1, S, D) and B_W_gate.shape == (D, F) and A_wk.shape == (D, DH)
    hbm = pl.BlockSpec(memory_space=pl.ANY)
    out = pl.pallas_call(
        kernel,
        in_specs=[hbm] * 9,
        out_specs=hbm,
        out_shape=jax.ShapeDtypeStruct((S, D), A_x.dtype),
        scratch_shapes=[
            pltpu.VMEM((4 * G + 1, KG // NB, FM * G * 128), BF16),
            pltpu.VMEM((4 * G + 1, KG // NB, FM * G * 128), BF16),
            pltpu.VMEM((4 * GM * G + 1, 16, D), BF16),
            pltpu.VMEM((NB, NPROD, MB // 2, KG), U32),
            pltpu.VMEM((NPROD, KG // 2, max(FFN_GROUPS[0::2]) * 256), U32),
            pltpu.VMEM((NPROD, KG // 2, max(FFN_GROUPS[1::2]) * 256), U32),
            pltpu.VMEM((NPROD, max(GROUPS[0::2]) * 64, KG), U32),
            pltpu.VMEM((NPROD, max(GROUPS[1::2]) * 64, KG), U32),
            pltpu.VMEM((S // 2, 128), U32),
            pltpu.VMEM((S // 128, DH // 2, 128), U32),
            pltpu.VMEM((S, 128), F32),
            pltpu.VMEM((S, 128), F32),
            pltpu.VMEM((S // 128 + 1, D // 2, 128), U32),
            pltpu.VMEM((NB, D, TQ), F32),
            pltpu.VMEM((24, 512), F32),
            pltpu.VMEM((6, 8, TQ), F32),
            pltpu.SMEM((4,), jnp.int32),
            pltpu.SemaphoreType.DMA((NB,)),
            pltpu.SemaphoreType.DMA((NQ * G,)),
            pltpu.SemaphoreType.DMA((3,)),
            pltpu.SemaphoreType.DMA((16,)),
            pltpu.SemaphoreType.DMA((2,)),
        ],
        compiler_params=pltpu.CompilerParams(vmem_limit_bytes=127 * 2**20),
        name="gated_mix",
    )(A_x.reshape(S, D), A_wq, A_wk.T, A_wv.T, A_wo.reshape(D // 128, 128, D),
      B_W_gate.reshape(G, KG, F), B_W_up.reshape(G, KG, F), B_W_down.reshape(F // 128, 128, D),
      gate_w.reshape(D // 128, 128))
    return out.reshape(A_x.shape)
```
